```python
import os as _os
_os.environ.setdefault('JAX_PLATFORMS', 'cpu')
import jax
import jax.numpy as jnp

def _softmax(x, axis=-1):
    return jax.nn.softmax(x, axis=axis)

def _gelu(x):
    return jax.nn.gelu(x, approximate=True)

def _silu(x):
    return jax.nn.silu(x)

def _sigmoid(x):
    return jax.nn.sigmoid(x)

def _layernorm(x, axis=-1, eps=1e-05):
    m = jnp.mean(x, axis=axis, keepdims=True)
    v = jnp.var(x, axis=axis, keepdims=True)
    return (x - m) / jnp.sqrt(v + eps)

def _scatter_add(tgt, idx, src, axis=0):
    return tgt.at[idx].add(src)

def _segment_sum(src, seg, n):
    return jax.ops.segment_sum(src, seg, n)

class _Rng:

    def __init__(self, key):
        self._k = key

    def _next(self):
        self._k, sub = jax.random.split(self._k)
        return sub

    def normal(self, shape):
        return jax.random.normal(self._next(), shape, dtype=jnp.bfloat16)

    def randint(self, lo, hi, shape):
        return jax.random.randint(self._next(), shape, lo, hi, dtype=jnp.int32)

    def uniform(self, shape, lo=0.0, hi=1.0):
        return jax.random.uniform(self._next(), shape, jnp.bfloat16, lo, hi)

    def permutation(self, n):
        return jax.random.permutation(self._next(), n)
kernel_name = 'gated_mix__mha_block__memory_aug_recurrent_mem_tr__prompt'

def setup_inputs():
    _rng = _Rng(jax.random.key(int.from_bytes(__import__("os").urandom(4), "little")))
    _w = lambda a: (lambda t: t.astype(jnp.bfloat16) if jnp.issubdtype(t.dtype, jnp.floating) else t)(jnp.asarray(a))

    def _A_setup():
        B, S, D, H = (1, 2048, 512, 32)
        return {'x': _w((lambda *s: _rng.normal(s) * 0.05)(B, S, D)), 'wqkv': _w((lambda *s: _rng.normal(s) * 0.8)(D, 3 * D)), 'wo': _w((lambda *s: _rng.normal(s) * 0.05)(D, D))}
    _A_in = _A_setup()

    def _B_setup():
        B, S, Dm = (1, 2048, 512)
        H, Dh = (32, 128)
        M, seg = (8, 32)
        seg = min(seg, S)
        S = S // seg * seg
        return {'x': _w((lambda *s: _rng.normal(s) * 0.05)(B, S, Dm)), 'mem0': _w((lambda *s: _rng.normal(s) * 0.8)(B, M, Dm)), 'Wq': _w((lambda *s: _rng.normal(s) * 1.6)(Dm, H, Dh) * Dm ** (-0.5)), 'Wk': _w((lambda *s: _rng.normal(s) * 1.6)(Dm, H, Dh) * Dm ** (-0.5)), 'Wv': _w((lambda *s: _rng.normal(s) * 0.8)(Dm, H, Dh) * Dm ** (-0.5)), 'Wo': _w((lambda *s: _rng.normal(s) * 0.8)(H, Dh, Dm) * (H * Dh) ** (-0.5)), 'seg_len': seg}
    _B_in = _B_setup()
    return {'A_x': _A_in['x'], 'A_wqkv': _A_in['wqkv'], 'A_wo': _A_in['wo'], 'B_x': _B_in['x'], 'B_mem0': _B_in['mem0'], 'B_Wq': _B_in['Wq'], 'B_Wk': _B_in['Wk'], 'B_Wv': _B_in['Wv'], 'B_Wo': _B_in['Wo'], 'B_seg_len': _B_in['seg_len'], 'gate_w': _w((lambda *s: _rng.normal(s) * 0.05)(512) * 16.0)}

def reference(A_x, A_wqkv, A_wo, B_x, B_mem0, B_Wq, B_Wk, B_Wv, B_Wo, B_seg_len, gate_w):

    def _A_ref(x, wqkv, wo):
        B, S, D = x.shape
        H = 32
        Dh = D // H
        qkv = (lambda x, *d: x.transpose(*d))((x @ wqkv).reshape(B, S, 3, H, Dh), 2, 0, 3, 1, 4)
        q, k, v = (qkv[0], qkv[1], qkv[2])
        scores = jnp.einsum('bhqd,bhkd->bhqk', q, k) * Dh ** (-0.5)
        p = _softmax(scores, axis=-1)
        o = jnp.einsum('bhqk,bhkd->bhqd', p, v)
        return (lambda x, *d: x.transpose(*d))(o, 0, 2, 1, 3).reshape(B, S, D) @ wo

    def _B_ref(x, mem0, Wq, Wk, Wv, Wo, seg_len):
        B, S, Dm = x.shape
        H, Dh = (Wq.shape[1], Wq.shape[2])
        M = mem0.shape[1]
        scale = Dh ** (-0.5)
        n_seg = S // seg_len
        L = M + seg_len
        idx = jnp.arange(L)
        mask = (idx[:, None] < M) | (idx[:, None] >= idx[None, :])
        mem = mem0
        outs = []
        for s in range(n_seg):
            xs = x[:, s * seg_len:(s + 1) * seg_len, :].copy()
            h = jnp.concatenate([mem, xs], axis=1)
            q = jnp.einsum('btd,dhe->bhte', h, Wq)
            k = jnp.einsum('btd,dhe->bhte', h, Wk)
            v = jnp.einsum('btd,dhe->bhte', h, Wv)
            scores = jnp.einsum('bhqe,bhke->bhqk', q, k) * scale
            scores = jnp.where(mask[None, None], scores, -1000000000.0)
            p = _softmax(scores, axis=-1)
            o = jnp.einsum('bhqk,bhke->bhqe', p, v)
            o = jnp.einsum('bhte,hed->btd', o, Wo)
            mem = o[:, :M, :].copy()
            outs.append(o[:, M:, :])
        return jnp.concatenate(outs, axis=1)
    x = A_x
    g = _sigmoid((x * gate_w).sum(-1, keepdims=True))
    a = _A_ref(x, A_wqkv, A_wo)
    b = _B_ref(x, B_mem0, B_Wq, B_Wk, B_Wv, B_Wo, B_seg_len)
    return g * a + (1 - g) * b
```

```python
import functools

import jax
import jax.numpy as jnp
import jax.experimental.pallas as pl
import jax.experimental.pallas.tpu as pltpu

bf16 = jnp.bfloat16
f32 = jnp.float32
u32 = jnp.uint32
LOG2E = 1.4426950408889634


def _kernel(x_ref, awqkv_ref, awo_ref, mem0_ref, wq_ref, wk_ref, wv_ref, wo_ref, gw_ref,
            out_ref,
            ka_ref, qT_ref, vT_ref, oT_ref, qm32_ref,
            b_ref, h48_ref, h32_ref, q_ref, k_ref, v_ref, oe_ref, oo_ref,
            wq2_ref, wk2_ref, wv2_ref, wo2_ref,
            *, S, D, HA, DHA, HB, DHB, SEG, TQ, TW, KB, HG, LA):
    NG = HB // HG
    GW = HG * DHB
    NK = S // KB
    NT = TQ // TW
    NTILES = NK * NT
    R = 48
    M = 8

    for c0 in range(0, HB * DHB, 512):
        wq2_ref[:, c0:c0 + 512] = pltpu.bitcast(wq_ref[:, c0:c0 + 512], u32)
        wk2_ref[:, c0:c0 + 512] = pltpu.bitcast(wk_ref[:, c0:c0 + 512], u32)
        wv2_ref[:, c0:c0 + 512] = pltpu.bitcast(wv_ref[:, c0:c0 + 512], u32)
        wo2_ref[c0 // 2:c0 // 2 + 256, :] = pltpu.bitcast(wo_ref[c0:c0 + 512, :], u32)

    x = x_ref[...]
    wqkv = awqkv_ref[...]
    qa = jnp.dot(x, wqkv[:, 0:D], preferred_element_type=f32).astype(bf16)
    ka_ref[...] = jnp.dot(x, wqkv[:, D:2 * D], preferred_element_type=f32).astype(bf16)
    va = jnp.dot(x, wqkv[:, 2 * D:3 * D], preferred_element_type=f32).astype(bf16)
    qT_ref[...] = (qa.astype(f32) * (DHA ** -0.5)).T.astype(bf16)
    vT_ref[...] = va.astype(f32).T.astype(bf16)
    rowg = jax.lax.broadcasted_iota(jnp.int32, (128, TQ), 0) // DHA

    h48_ref[32:40, :] = mem0_ref[...]
    scale = DHB ** -0.5
    cB = scale * LOG2E

    def classify(idx, parity):
        if parity == 0:
            return idx, (idx >= 32) & (idx < 40), idx < 40
        t = jnp.where(idx < 16, idx + 16, jnp.where(idx >= 40, idx - 40, idx - 16))
        return t, (idx >= 16) & (idx < 24), (idx < 32) | (idx >= 40)

    ri = jax.lax.broadcasted_iota(jnp.int32, (R, R), 0)
    ci = jax.lax.broadcasted_iota(jnp.int32, (R, R), 1)
    valids, fills = [], []
    for parity in (0, 1):
        ti, mi, oki = classify(ri, parity)
        tj, mj, okj = classify(ci, parity)
        valids.append(okj & (mj | mi | (~oki) | (tj <= ti)))
        fills.append(jnp.where(okj, -1e9 / scale, -3e38).astype(f32))
    lowhalf = jax.lax.broadcasted_iota(jnp.int32, (16, GW), 0) < 8

    def make_a_unit(h, qb):
        g_ = h // (128 // DHA)
        r_ = h % (128 // DHA)
        qstart = qb * TQ
        gstart = pl.multiple_of(g_ * 128, 128)
        hstart = pl.multiple_of(h * DHA, DHA)
        A = {'issued': 0, 'done': 0, 'S': {}, 'm': [None] * NT, 'l': [None] * NT, 'acc': [None] * NT}

        def issue():
            j = A['issued']
            kb, qt = divmod(j, NT)
            A['S'][j] = jnp.dot(ka_ref[kb * KB:(kb + 1) * KB, pl.ds(gstart, 128)],
                                pltpu.bitcast(qm32_ref[:, qt * TW:(qt + 1) * TW], bf16),
                                preferred_element_type=f32)
            A['issued'] = j + 1

        def a_init():
            qg = qT_ref[pl.ds(gstart, 128), qstart:qstart + TQ]
            qm32_ref[...] = pltpu.bitcast(jnp.where(rowg == r_, qg.astype(f32), 0.0).astype(bf16), u32)
            for _ in range(LA):
                issue()

        def a_tile():
            j = A['done']
            kb, qt = divmod(j, NT)
            if A['issued'] < NTILES:
                issue()
            s = A['S'].pop(j)
            bm = jnp.max(s, axis=0, keepdims=True)
            vT = vT_ref[pl.ds(hstart, DHA), kb * KB:(kb + 1) * KB]
            if kb == 0:
                m_new = bm
                e = jnp.exp(s - m_new)
                A['l'][qt] = jnp.sum(e, axis=0, keepdims=True)
                A['acc'][qt] = jnp.dot(vT, e.astype(bf16), preferred_element_type=f32)
            else:
                m_new = jnp.maximum(A['m'][qt], bm)
                alpha = jnp.exp(A['m'][qt] - m_new)
                e = jnp.exp(s - m_new)
                A['l'][qt] = alpha * A['l'][qt] + jnp.sum(e, axis=0, keepdims=True)
                A['acc'][qt] = alpha * A['acc'][qt] + jnp.dot(vT, e.astype(bf16), preferred_element_type=f32)
            A['m'][qt] = m_new
            A['done'] = j + 1

        def a_chunk():
            for _ in range(NT):
                a_tile()

        def a_final():
            assert A['done'] == NTILES
            for qt in range(NT):
                oT_ref[pl.ds(hstart, DHA), qstart + qt * TW:qstart + (qt + 1) * TW] = A['acc'][qt] / A['l'][qt]

        return a_init, a_chunk, a_final

    def half_step(parity, base, a_unit):
        a_init, a_chunk, a_final = a_unit
        valid, fill = valids[parity], fills[parity]
        o_ref = oe_ref if parity == 0 else oo_ref
        RP = 48 if parity == 0 else 32
        Bs = {'acc': None}

        def proj1(g, which):
            w_ref, dst_ref = {'q': (wq2_ref, q_ref), 'k': (wk2_ref, k_ref), 'v': (wv2_ref, v_ref)}[which]
            cs = slice(g * GW, (g + 1) * GW)
            dst_ref[0:RP, cs] = jnp.dot(Bs['hh'], pltpu.bitcast(w_ref[:, cs], bf16),
                                        preferred_element_type=f32).astype(bf16)

        def heads(g):
            return range(g * HG, (g + 1) * HG)

        def b_scores(g):
            Bs['sc'] = [jax.lax.dot_general(q_ref[:, hd * DHB:(hd + 1) * DHB], k_ref[:, hd * DHB:(hd + 1) * DHB],
                                            (((1,), (1,)), ((), ())), preferred_element_type=f32)
                        for hd in heads(g)]

        def b_softmax():
            ps, rs = [], []
            for sc in Bs['sc']:
                sc = jnp.where(valid, sc, fill)
                m = jnp.max(sc, axis=-1, keepdims=True)
                e = jnp.exp2((sc - m) * cB)
                l = jnp.sum(e, axis=-1, keepdims=True)
                r0 = pl.reciprocal(l, approx=True)
                r0 = r0 * (2.0 - l * r0)
                r0 = r0 * (2.0 - l * r0)
                ps.append(e.astype(bf16))
                rs.append(r0)
            Bs['p'], Bs['r'] = ps, rs

        def b_pv(g):
            Bs['oh'] = [jnp.dot(Bs['p'][i], v_ref[:, hd * DHB:(hd + 1) * DHB], preferred_element_type=f32)
                        for i, hd in enumerate(heads(g))]

        def b_norm(g):
            for i, hd in enumerate(heads(g)):
                o_ref[:, hd * DHB:(hd + 1) * DHB] = (Bs['oh'][i] * Bs['r'][i]).astype(bf16)

        def b_wo(g):
            cs = slice(g * GW, (g + 1) * GW)
            if parity == 0:
                lhs = jnp.concatenate([oe_ref[16:32, cs],
                                       jnp.where(lowhalf, oe_ref[32:48, cs], oe_ref[0:16, cs])], axis=0)
            else:
                lhs = jnp.concatenate([oo_ref[0:32, cs],
                                       jnp.where(lowhalf, oe_ref[0:16, cs], oo_ref[32:48, cs])], axis=0)
            part = jnp.dot(lhs, pltpu.bitcast(wo2_ref[g * GW // 2:(g + 1) * GW // 2, :], bf16),
                           preferred_element_type=f32)
            Bs['acc'] = part if Bs['acc'] is None else Bs['acc'] + part

        a_init()
        if parity == 0:
            h48_ref[0:32, :] = x_ref[pl.ds(base, 32), :]
            h48_ref[40:48, :] = x_ref[pl.ds(base + 32, 8), :]
            Bs['hh'] = h48_ref[...]
        else:
            h32_ref[0:16, :] = x_ref[pl.ds(base + 48, 16), :]
            h32_ref[24:32, :] = x_ref[pl.ds(base + 40, 8), :]
            Bs['hh'] = h32_ref[...]
        na_mid = NK - 4
        a_chunk()
        proj1(0, 'q'); proj1(0, 'k'); proj1(0, 'v')
        done_mid = 0
        for g in range(NG):
            last = g + 1 == NG
            b_scores(g)
            if not last:
                proj1(g + 1, 'q')
            else:
                a_chunk()
            b_softmax()
            b_pv(g)
            if not last:
                proj1(g + 1, 'k')
            else:
                a_chunk()
            b_norm(g)
            b_wo(g)
            if not last:
                proj1(g + 1, 'v')
                tgt = (na_mid * (g + 1)) // (NG - 1)
                while done_mid < tgt:
                    a_chunk()
                    done_mid += 1
            else:
                a_chunk()
        outb = Bs['acc'].astype(bf16)
        if parity == 0:
            b_ref[pl.ds(base + 16, 16), :] = outb[0:16, :]
            h32_ref[16:24, :] = outb[16:24, :]
            b_ref[pl.ds(base + 8, 8), :] = outb[24:32, :]
        else:
            b_ref[pl.ds(base + 48, 16), :] = outb[0:16, :]
            h48_ref[32:40, :] = outb[16:24, :]
            b_ref[pl.ds(base + 40, 8), :] = outb[24:32, :]
            b_ref[pl.ds(base, 8), :] = outb[32:40, :]
            b_ref[pl.ds(base + 32, 8), :] = outb[40:48, :]
        a_final()

    def body(t, carry):
        base = pl.multiple_of(t * (2 * SEG), 2 * SEG)
        half_step(0, base, make_a_unit(t, 0))
        half_step(1, base, make_a_unit(t, 1))
        return carry

    jax.lax.fori_loop(0, S // (2 * SEG), body, 0)

    oa = oT_ref[...].T.astype(bf16)
    a = jnp.dot(oa, awo_ref[...], preferred_element_type=f32).astype(bf16).astype(f32)
    logit = jnp.sum(x_ref[...].astype(f32) * gw_ref[...].astype(f32), axis=-1, keepdims=True)
    gate = 1.0 / (1.0 + jnp.exp(-logit))
    out_ref[...] = (gate * a + (1.0 - gate) * b_ref[...].astype(f32)).astype(bf16)


@functools.partial(jax.jit, static_argnames=("B_seg_len",))
def pallas_gated_mix__mha_block__memory_aug_recurrent_mem_tr__prompt_kernel(
    A_x: jax.Array,
    A_wqkv: jax.Array,
    A_wo: jax.Array,
    B_x: jax.Array,
    B_mem0: jax.Array,
    B_Wq: jax.Array,
    B_Wk: jax.Array,
    B_Wv: jax.Array,
    B_Wo: jax.Array,
    B_seg_len: int,
    gate_w: jax.Array,
):
    Bsz, S, D = A_x.shape
    HA, DHA = 32, D // 32
    HB, DHB = B_Wq.shape[1], B_Wq.shape[2]
    M = B_mem0.shape[1]
    SEG = int(B_seg_len)
    TQ, TW, KB, HG, LA = 1024, 128, 128, 8, 12
    assert Bsz == 1 and DHA == 16 and DHB == 128 and M == 8 and SEG == 32
    assert S == 2 * TQ and HA * (S // TQ) == S // SEG and HB % HG == 0
    R = 48

    x = A_x.reshape(S, D)
    mem0 = B_mem0.reshape(M, D)
    wq = B_Wq.reshape(D, HB * DHB)
    wk = B_Wk.reshape(D, HB * DHB)
    wv = B_Wv.reshape(D, HB * DHB)
    wo = B_Wo.reshape(HB * DHB, D)
    gw = gate_w.reshape(1, D)

    kernel = functools.partial(_kernel, S=S, D=D, HA=HA, DHA=DHA, HB=HB, DHB=DHB, SEG=SEG,
                               TQ=TQ, TW=TW, KB=KB, HG=HG, LA=LA)
    out = pl.pallas_call(
        kernel,
        out_shape=jax.ShapeDtypeStruct((S, D), bf16),
        scratch_shapes=[
            pltpu.VMEM((S, D), bf16),
            pltpu.VMEM((D, S), bf16),
            pltpu.VMEM((D, S), bf16),
            pltpu.VMEM((D, S), f32),
            pltpu.VMEM((64, TQ), u32),
            pltpu.VMEM((S, D), bf16),
            pltpu.VMEM((48, D), bf16),
            pltpu.VMEM((32, D), bf16),
            pltpu.VMEM((R, HB * DHB), bf16),
            pltpu.VMEM((R, HB * DHB), bf16),
            pltpu.VMEM((R, HB * DHB), bf16),
            pltpu.VMEM((R, HB * DHB), bf16),
            pltpu.VMEM((R, HB * DHB), bf16),
            pltpu.VMEM((D // 2, HB * DHB), u32),
            pltpu.VMEM((D // 2, HB * DHB), u32),
            pltpu.VMEM((D // 2, HB * DHB), u32),
            pltpu.VMEM((HB * DHB // 2, D), u32),
        ],
        compiler_params=pltpu.CompilerParams(vmem_limit_bytes=100 * 1024 * 1024),
    )(x, A_wqkv, A_wo, mem0, wq, wk, wv, wo, gw)
    return out.reshape(Bsz, S, D)
```

```python
import functools

import jax
import jax.numpy as jnp
import jax.experimental.pallas as pl
import jax.experimental.pallas.tpu as pltpu

bf16 = jnp.bfloat16
f32 = jnp.float32
u32 = jnp.uint32
LOG2E = 1.4426950408889634


def _kernel(x_hbm, awqkv_hbm, awo_hbm, mem0_ref, wq_hbm, wk_hbm, wv_hbm, wo_hbm, gw_ref,
            out_ref,
            x_ref, awqkv_ref, awo_ref, wq_ref, wk_ref, wv_ref, wo_ref, sems,
            ka_ref, qT_ref, vT_ref, oT_ref, qm32_ref,
            b_ref, h48_ref, h32_ref, q_ref, k_ref, v_ref, oe_ref, oo_ref,
            wq2_ref, wk2_ref, wv2_ref, wo2_ref,
            *, S, D, HA, DHA, HB, DHB, SEG, TQ, TW, KB, HG, LA):
    NG = HB // HG
    GW = HG * DHB
    NK = S // KB
    NT = TQ // TW
    NTILES = NK * NT
    R = 48
    M = 8

    copies = [pltpu.make_async_copy(src, dst, sems.at[i]) for i, (src, dst) in enumerate([
        (x_hbm, x_ref), (awqkv_hbm, awqkv_ref), (wq_hbm, wq_ref), (wk_hbm, wk_ref),
        (wv_hbm, wv_ref), (wo_hbm, wo_ref), (awo_hbm, awo_ref)])]
    cp_x, cp_wqkv, cp_wq, cp_wk, cp_wv, cp_wo, cp_awo = copies
    cp_x.start()
    cp_wqkv.start()
    cp_x.wait()
    cp_wqkv.wait()
    for cp in (cp_wq, cp_wk, cp_wv, cp_wo, cp_awo):
        cp.start()

    def repack(raw_ref, dst_ref):
        raw32 = raw_ref.bitcast(u32)
        for j in range(HB // 2):
            for i0 in range(0, D // 2, 64):
                ev = raw32[pl.ds((2 * i0) * (HB // 2) + j, 64, stride=HB), :]
                od = raw32[pl.ds((2 * i0 + 1) * (HB // 2) + j, 64, stride=HB), :]
                dst_ref[i0:i0 + 64, (2 * j) * DHB:(2 * j + 1) * DHB] = (ev & jnp.uint32(0xFFFF)) | (od << 16)
                dst_ref[i0:i0 + 64, (2 * j + 1) * DHB:(2 * j + 2) * DHB] = (ev >> 16) | (od & jnp.uint32(0xFFFF0000))

    x = x_ref[...]
    qa = jnp.dot(x, awqkv_ref[:, 0:D], preferred_element_type=f32).astype(bf16)
    cp_wq.wait()
    repack(wq_ref, wq2_ref)
    ka_ref[...] = jnp.dot(x, awqkv_ref[:, D:2 * D], preferred_element_type=f32).astype(bf16)
    cp_wk.wait()
    repack(wk_ref, wk2_ref)
    va = jnp.dot(x, awqkv_ref[:, 2 * D:3 * D], preferred_element_type=f32).astype(bf16)
    qT_ref[...] = (qa.astype(f32) * (DHA ** -0.5)).T.astype(bf16)
    cp_wv.wait()
    repack(wv_ref, wv2_ref)
    vT_ref[...] = va.astype(f32).T.astype(bf16)
    cp_wo.wait()
    for c0 in range(0, HB * DHB, 512):
        wo2_ref[c0 // 2:c0 // 2 + 256, :] = pltpu.bitcast(wo_ref[c0:c0 + 512, :], u32)
    rowg = jax.lax.broadcasted_iota(jnp.int32, (128, TQ), 0) // DHA

    h48_ref[32:40, :] = mem0_ref[...]
    scale = DHB ** -0.5
    cB = scale * LOG2E

    def classify(idx, parity):
        if parity == 0:
            return idx, (idx >= 32) & (idx < 40), idx < 40
        t = jnp.where(idx < 16, idx + 16, jnp.where(idx >= 40, idx - 40, idx - 16))
        return t, (idx >= 16) & (idx < 24), (idx < 32) | (idx >= 40)

    ri = jax.lax.broadcasted_iota(jnp.int32, (R, R), 0)
    ci = jax.lax.broadcasted_iota(jnp.int32, (R, R), 1)
    valids, fills = [], []
    for parity in (0, 1):
        ti, mi, oki = classify(ri, parity)
        tj, mj, okj = classify(ci, parity)
        valids.append(okj & (mj | mi | (~oki) | (tj <= ti)))
        fills.append(jnp.where(okj, -1e9 / scale, -3e38).astype(f32))
    lowhalf = jax.lax.broadcasted_iota(jnp.int32, (16, GW), 0) < 8

    def make_a_unit(h, qb):
        g_ = h // (128 // DHA)
        r_ = h % (128 // DHA)
        qstart = qb * TQ
        gstart = pl.multiple_of(g_ * 128, 128)
        hstart = pl.multiple_of(h * DHA, DHA)
        A = {'issued': 0, 'done': 0, 'S': {}, 'm': [None] * NT, 'l': [None] * NT, 'acc': [None] * NT}

        def issue():
            j = A['issued']
            kb, qt = divmod(j, NT)
            A['S'][j] = jnp.dot(ka_ref[kb * KB:(kb + 1) * KB, pl.ds(gstart, 128)],
                                pltpu.bitcast(qm32_ref[:, qt * TW:(qt + 1) * TW], bf16),
                                preferred_element_type=f32)
            A['issued'] = j + 1

        def a_init():
            qg = qT_ref[pl.ds(gstart, 128), qstart:qstart + TQ]
            qm32_ref[...] = pltpu.bitcast(jnp.where(rowg == r_, qg.astype(f32), 0.0).astype(bf16), u32)
            for _ in range(LA):
                issue()

        def a_tile():
            j = A['done']
            kb, qt = divmod(j, NT)
            if A['issued'] < NTILES:
                issue()
            s = A['S'].pop(j)
            bm = jnp.max(s, axis=0, keepdims=True)
            vT = vT_ref[pl.ds(hstart, DHA), kb * KB:(kb + 1) * KB]
            if kb == 0:
                m_new = bm
                e = jnp.exp(s - m_new)
                A['l'][qt] = jnp.sum(e, axis=0, keepdims=True)
                A['acc'][qt] = jnp.dot(vT, e.astype(bf16), preferred_element_type=f32)
            else:
                m_new = jnp.maximum(A['m'][qt], bm)
                alpha = jnp.exp(A['m'][qt] - m_new)
                e = jnp.exp(s - m_new)
                A['l'][qt] = alpha * A['l'][qt] + jnp.sum(e, axis=0, keepdims=True)
                A['acc'][qt] = alpha * A['acc'][qt] + jnp.dot(vT, e.astype(bf16), preferred_element_type=f32)
            A['m'][qt] = m_new
            A['done'] = j + 1

        def a_chunk():
            for _ in range(NT):
                a_tile()

        def a_final():
            assert A['done'] == NTILES
            for qt in range(NT):
                oT_ref[pl.ds(hstart, DHA), qstart + qt * TW:qstart + (qt + 1) * TW] = A['acc'][qt] / A['l'][qt]

        return a_init, a_chunk, a_final

    def half_step(parity, base, a_unit):
        a_init, a_chunk, a_final = a_unit
        valid, fill = valids[parity], fills[parity]
        o_ref = oe_ref if parity == 0 else oo_ref
        RP = 48 if parity == 0 else 32
        Bs = {'acc': None}

        def proj1(g, which):
            w_ref, dst_ref = {'q': (wq2_ref, q_ref), 'k': (wk2_ref, k_ref), 'v': (wv2_ref, v_ref)}[which]
            cs = slice(g * GW, (g + 1) * GW)
            dst_ref[0:RP, cs] = jnp.dot(Bs['hh'], pltpu.bitcast(w_ref[:, cs], bf16),
                                        preferred_element_type=f32).astype(bf16)

        def heads(g):
            return range(g * HG, (g + 1) * HG)

        def b_scores(g):
            Bs['sc'] = [jax.lax.dot_general(q_ref[:, hd * DHB:(hd + 1) * DHB], k_ref[:, hd * DHB:(hd + 1) * DHB],
                                            (((1,), (1,)), ((), ())), preferred_element_type=f32)
                        for hd in heads(g)]

        def b_softmax():
            ps, rs = [], []
            for sc in Bs['sc']:
                sc = jnp.where(valid, sc, fill)
                m = jnp.max(sc, axis=-1, keepdims=True)
                e = jnp.exp2((sc - m) * cB)
                l = jnp.sum(e, axis=-1, keepdims=True)
                r0 = pl.reciprocal(l, approx=True)
                r0 = r0 * (2.0 - l * r0)
                r0 = r0 * (2.0 - l * r0)
                ps.append(e.astype(bf16))
                rs.append(r0)
            Bs['p'], Bs['r'] = ps, rs

        def b_pv(g):
            Bs['oh'] = [jnp.dot(Bs['p'][i], v_ref[:, hd * DHB:(hd + 1) * DHB], preferred_element_type=f32)
                        for i, hd in enumerate(heads(g))]

        def b_norm(g):
            for i, hd in enumerate(heads(g)):
                o_ref[:, hd * DHB:(hd + 1) * DHB] = (Bs['oh'][i] * Bs['r'][i]).astype(bf16)

        def b_wo(g):
            cs = slice(g * GW, (g + 1) * GW)
            if parity == 0:
                lhs = jnp.concatenate([oe_ref[16:32, cs],
                                       jnp.where(lowhalf, oe_ref[32:48, cs], oe_ref[0:16, cs])], axis=0)
            else:
                lhs = jnp.concatenate([oo_ref[0:32, cs],
                                       jnp.where(lowhalf, oe_ref[0:16, cs], oo_ref[32:48, cs])], axis=0)
            part = jnp.dot(lhs, pltpu.bitcast(wo2_ref[g * GW // 2:(g + 1) * GW // 2, :], bf16),
                           preferred_element_type=f32)
            Bs['acc'] = part if Bs['acc'] is None else Bs['acc'] + part

        a_init()
        if parity == 0:
            h48_ref[0:32, :] = x_ref[pl.ds(base, 32), :]
            h48_ref[40:48, :] = x_ref[pl.ds(base + 32, 8), :]
            Bs['hh'] = h48_ref[...]
        else:
            h32_ref[0:16, :] = x_ref[pl.ds(base + 48, 16), :]
            h32_ref[24:32, :] = x_ref[pl.ds(base + 40, 8), :]
            Bs['hh'] = h32_ref[...]
        na_mid = NK - 4
        a_chunk()
        proj1(0, 'q'); proj1(0, 'k'); proj1(0, 'v')
        done_mid = 0
        for g in range(NG):
            last = g + 1 == NG
            b_scores(g)
            if not last:
                proj1(g + 1, 'q')
            else:
                a_chunk()
            b_softmax()
            b_pv(g)
            if not last:
                proj1(g + 1, 'k')
            else:
                a_chunk()
            b_norm(g)
            b_wo(g)
            if not last:
                proj1(g + 1, 'v')
                tgt = (na_mid * (g + 1)) // (NG - 1)
                while done_mid < tgt:
                    a_chunk()
                    done_mid += 1
            else:
                a_chunk()
        outb = Bs['acc'].astype(bf16)
        if parity == 0:
            b_ref[pl.ds(base + 16, 16), :] = outb[0:16, :]
            h32_ref[16:24, :] = outb[16:24, :]
            b_ref[pl.ds(base + 8, 8), :] = outb[24:32, :]
        else:
            b_ref[pl.ds(base + 48, 16), :] = outb[0:16, :]
            h48_ref[32:40, :] = outb[16:24, :]
            b_ref[pl.ds(base + 40, 8), :] = outb[24:32, :]
            b_ref[pl.ds(base, 8), :] = outb[32:40, :]
            b_ref[pl.ds(base + 32, 8), :] = outb[40:48, :]
        a_final()

    def body(t, carry):
        base = pl.multiple_of(t * (2 * SEG), 2 * SEG)
        half_step(0, base, make_a_unit(t, 0))
        half_step(1, base, make_a_unit(t, 1))
        return carry

    jax.lax.fori_loop(0, S // (2 * SEG), body, 0)

    oa = oT_ref[...].T.astype(bf16)
    cp_awo.wait()
    a = jnp.dot(oa, awo_ref[...], preferred_element_type=f32).astype(bf16).astype(f32)
    logit = jnp.sum(x_ref[...].astype(f32) * gw_ref[...].astype(f32), axis=-1, keepdims=True)
    gate = 1.0 / (1.0 + jnp.exp(-logit))
    out_ref[...] = (gate * a + (1.0 - gate) * b_ref[...].astype(f32)).astype(bf16)


@functools.partial(jax.jit, static_argnames=("B_seg_len",))
def pallas_gated_mix__mha_block__memory_aug_recurrent_mem_tr__prompt_kernel(
    A_x: jax.Array,
    A_wqkv: jax.Array,
    A_wo: jax.Array,
    B_x: jax.Array,
    B_mem0: jax.Array,
    B_Wq: jax.Array,
    B_Wk: jax.Array,
    B_Wv: jax.Array,
    B_Wo: jax.Array,
    B_seg_len: int,
    gate_w: jax.Array,
):
    Bsz, S, D = A_x.shape
    HA, DHA = 32, D // 32
    HB, DHB = B_Wq.shape[1], B_Wq.shape[2]
    M = B_mem0.shape[1]
    SEG = int(B_seg_len)
    TQ, TW, KB, HG, LA = 1024, 128, 128, 8, 12
    assert Bsz == 1 and DHA == 16 and DHB == 128 and M == 8 and SEG == 32
    assert S == 2 * TQ and HA * (S // TQ) == S // SEG and HB % HG == 0
    R = 48

    x = A_x.reshape(S, D)
    mem0 = B_mem0.reshape(M, D)
    wq = B_Wq.reshape(D * HB, DHB)
    wk = B_Wk.reshape(D * HB, DHB)
    wv = B_Wv.reshape(D * HB, DHB)
    wo = B_Wo.reshape(HB * DHB, D)
    gw = gate_w.reshape(1, D)

    kernel = functools.partial(_kernel, S=S, D=D, HA=HA, DHA=DHA, HB=HB, DHB=DHB, SEG=SEG,
                               TQ=TQ, TW=TW, KB=KB, HG=HG, LA=LA)
    hbm = pl.BlockSpec(memory_space=pl.ANY)
    vmem = pl.BlockSpec(memory_space=pltpu.VMEM)
    out = pl.pallas_call(
        kernel,
        out_shape=jax.ShapeDtypeStruct((S, D), bf16),
        in_specs=[hbm, hbm, hbm, vmem, hbm, hbm, hbm, hbm, vmem],
        scratch_shapes=[
            pltpu.VMEM((S, D), bf16),
            pltpu.VMEM((D, 3 * D), bf16),
            pltpu.VMEM((D, D), bf16),
            pltpu.VMEM((D * HB, DHB), bf16),
            pltpu.VMEM((D * HB, DHB), bf16),
            pltpu.VMEM((D * HB, DHB), bf16),
            pltpu.VMEM((HB * DHB, D), bf16),
            pltpu.SemaphoreType.DMA((7,)),
            pltpu.VMEM((S, D), bf16),
            pltpu.VMEM((D, S), bf16),
            pltpu.VMEM((D, S), bf16),
            pltpu.VMEM((D, S), f32),
            pltpu.VMEM((64, TQ), u32),
            pltpu.VMEM((S, D), bf16),
            pltpu.VMEM((48, D), bf16),
            pltpu.VMEM((32, D), bf16),
            pltpu.VMEM((R, HB * DHB), bf16),
            pltpu.VMEM((R, HB * DHB), bf16),
            pltpu.VMEM((R, HB * DHB), bf16),
            pltpu.VMEM((R, HB * DHB), bf16),
            pltpu.VMEM((R, HB * DHB), bf16),
            pltpu.VMEM((D // 2, HB * DHB), u32),
            pltpu.VMEM((D // 2, HB * DHB), u32),
            pltpu.VMEM((D // 2, HB * DHB), u32),
            pltpu.VMEM((HB * DHB // 2, D), u32),
        ],
        compiler_params=pltpu.CompilerParams(vmem_limit_bytes=100 * 1024 * 1024),
    )(x, A_wqkv, A_wo, mem0, wq, wk, wv, wo, gw)
    return out.reshape(Bsz, S, D)
```

```python
import functools

import jax
import jax.numpy as jnp
import jax.experimental.pallas as pl
import jax.experimental.pallas.tpu as pltpu

bf16 = jnp.bfloat16
f32 = jnp.float32
u32 = jnp.uint32
LOG2E = 1.4426950408889634


def _kernel(x_hbm, awqkv_hbm, awo_hbm, mem0_ref, wq_hbm, wk_hbm, wv_hbm, wo_hbm, gw_ref,
            out_ref,
            x_ref, awqkv_ref, awo_ref, wq_ref, wk_ref, wv_ref, wo_ref, sems,
            ka_ref, qT_ref, vT_ref, oT_ref, qm32e_ref, qm32o_ref,
            b_ref, h48_ref, h32_ref, q_ref, k_ref, v_ref, oe_ref, oo_ref,
            wq2_ref, wk2_ref, wv2_ref, wo2_ref,
            *, S, D, HA, DHA, HB, DHB, SEG, TQ, TW, KB, HG, LA, PW, A_HEAD, A_TAIL):
    NG = HB // HG
    GW = HG * DHB
    NK = S // KB
    NT = TQ // TW
    NTILES = NK * NT
    R = 48
    M = 8

    copies = [pltpu.make_async_copy(src, dst, sems.at[i]) for i, (src, dst) in enumerate([
        (x_hbm, x_ref), (awqkv_hbm, awqkv_ref), (wq_hbm, wq_ref), (wk_hbm, wk_ref),
        (wv_hbm, wv_ref), (wo_hbm, wo_ref), (awo_hbm, awo_ref)])]
    cp_x, cp_wqkv, cp_wq, cp_wk, cp_wv, cp_wo, cp_awo = copies
    cp_x.start()
    cp_wqkv.start()
    cp_x.wait()
    cp_wqkv.wait()
    for cp in (cp_wq, cp_wk, cp_wv, cp_wo, cp_awo):
        cp.start()

    def repack(raw_ref, dst_ref):
        raw32 = raw_ref.bitcast(u32)
        for j in range(HB // 2):
            for i0 in range(0, D // 2, 64):
                ev = raw32[pl.ds((2 * i0) * (HB // 2) + j, 64, stride=HB), :]
                od = raw32[pl.ds((2 * i0 + 1) * (HB // 2) + j, 64, stride=HB), :]
                dst_ref[i0:i0 + 64, (2 * j) * DHB:(2 * j + 1) * DHB] = (ev & jnp.uint32(0xFFFF)) | (od << 16)
                dst_ref[i0:i0 + 64, (2 * j + 1) * DHB:(2 * j + 2) * DHB] = (ev >> 16) | (od & jnp.uint32(0xFFFF0000))

    x = x_ref[...]
    qa = jnp.dot(x, awqkv_ref[:, 0:D], preferred_element_type=f32).astype(bf16)
    cp_wq.wait()
    repack(wq_ref, wq2_ref)
    ka_ref[...] = jnp.dot(x, awqkv_ref[:, D:2 * D], preferred_element_type=f32).astype(bf16)
    cp_wk.wait()
    repack(wk_ref, wk2_ref)
    va = jnp.dot(x, awqkv_ref[:, 2 * D:3 * D], preferred_element_type=f32).astype(bf16)
    qT_ref[...] = (qa.astype(f32) * (DHA ** -0.5)).T.astype(bf16)
    cp_wv.wait()
    repack(wv_ref, wv2_ref)
    vT_ref[...] = va.astype(f32).T.astype(bf16)
    cp_wo.wait()
    for c0 in range(0, HB * DHB, 512):
        wo2_ref[c0 // 2:c0 // 2 + 256, :] = pltpu.bitcast(wo_ref[c0:c0 + 512, :], u32)
    rowg = jax.lax.broadcasted_iota(jnp.int32, (128, TQ), 0) // DHA

    h48_ref[32:40, :] = mem0_ref[...]
    scale = DHB ** -0.5
    cB = scale * LOG2E

    def classify(idx, parity):
        if parity == 0:
            return idx, (idx >= 32) & (idx < 40), idx < 40
        t = jnp.where(idx < 16, idx + 16, jnp.where(idx >= 40, idx - 40, idx - 16))
        return t, (idx >= 16) & (idx < 24), (idx < 32) | (idx >= 40)

    ri = jax.lax.broadcasted_iota(jnp.int32, (R, R), 0)
    ci = jax.lax.broadcasted_iota(jnp.int32, (R, R), 1)
    valids, fills = [], []
    for parity in (0, 1):
        ti, mi, oki = classify(ri, parity)
        tj, mj, okj = classify(ci, parity)
        valids.append(okj & (mj | mi | (~oki) | (tj <= ti)))
        fills.append(jnp.where(okj, -1e9 / scale, -3e38).astype(f32))
    lowhalf = jax.lax.broadcasted_iota(jnp.int32, (16, GW), 0) < 8

    def build_qm(h, qb):
        g_ = h // (128 // DHA)
        r_ = h % (128 // DHA)
        gstart = pl.multiple_of(g_ * 128, 128)
        qg = qT_ref[pl.ds(gstart, 128), qb * TQ:(qb + 1) * TQ]
        qm32_ref = qm32e_ref if qb == 0 else qm32o_ref
        qm32_ref[...] = pltpu.bitcast(jnp.where(rowg == r_, qg.astype(f32), 0.0).astype(bf16), u32)

    def make_a_unit(h, qb):
        g_ = h // (128 // DHA)
        qstart = qb * TQ
        gstart = pl.multiple_of(g_ * 128, 128)
        hstart = pl.multiple_of(h * DHA, DHA)
        qm32_ref = qm32e_ref if qb == 0 else qm32o_ref
        A = {'issued': 0, 'done': 0, 'S': {}, 'm': [None] * NT, 'l': [None] * NT, 'acc': [None] * NT}

        def issue():
            j = A['issued']
            kb, qt = divmod(j, NT)
            A['S'][j] = jnp.dot(ka_ref[kb * KB:(kb + 1) * KB, pl.ds(gstart, 128)],
                                pltpu.bitcast(qm32_ref[:, qt * TW:(qt + 1) * TW], bf16),
                                preferred_element_type=f32)
            A['issued'] = j + 1

        def a_init():
            for _ in range(LA):
                issue()

        def a_tile():
            j = A['done']
            kb, qt = divmod(j, NT)
            if A['issued'] < NTILES:
                issue()
            s = A['S'].pop(j)
            bm = jnp.max(s, axis=0, keepdims=True)
            vT = vT_ref[pl.ds(hstart, DHA), kb * KB:(kb + 1) * KB]
            if kb == 0:
                m_new = bm
                e = jnp.exp(s - m_new)
                A['l'][qt] = jnp.sum(e, axis=0, keepdims=True)
                A['acc'][qt] = jnp.dot(vT, e.astype(bf16), preferred_element_type=f32)
            else:
                m_new = jnp.maximum(A['m'][qt], bm)
                alpha = jnp.exp(A['m'][qt] - m_new)
                e = jnp.exp(s - m_new)
                A['l'][qt] = alpha * A['l'][qt] + jnp.sum(e, axis=0, keepdims=True)
                A['acc'][qt] = alpha * A['acc'][qt] + jnp.dot(vT, e.astype(bf16), preferred_element_type=f32)
            A['m'][qt] = m_new
            A['done'] = j + 1

        def a_tiles(n):
            for _ in range(n):
                if A['done'] < NTILES:
                    a_tile()

        def a_final():
            assert A['done'] == NTILES
            for qt in range(NT):
                oT_ref[pl.ds(hstart, DHA), qstart + qt * TW:qstart + (qt + 1) * TW] = A['acc'][qt] / A['l'][qt]

        return a_init, a_tiles, a_final

    def half_step(parity, base, a_unit, prep_next):
        a_init, a_tiles, a_final = a_unit
        valid, fill = valids[parity], fills[parity]
        o_ref = oe_ref if parity == 0 else oo_ref
        RP = 48 if parity == 0 else 32
        Bs = {'acc': None}

        def proj1(g, which, piece):
            w_ref, dst_ref = {'q': (wq2_ref, q_ref), 'k': (wk2_ref, k_ref), 'v': (wv2_ref, v_ref)}[which]
            cs = slice(g * GW + piece * PW, g * GW + (piece + 1) * PW)
            dst_ref[0:RP, cs] = jnp.dot(Bs['hh'], pltpu.bitcast(w_ref[:, cs], bf16),
                                        preferred_element_type=f32).astype(bf16)

        def heads(g):
            return range(g * HG, (g + 1) * HG)

        def b_scores(g):
            Bs['sc'] = [jax.lax.dot_general(q_ref[:, hd * DHB:(hd + 1) * DHB], k_ref[:, hd * DHB:(hd + 1) * DHB],
                                            (((1,), (1,)), ((), ())), preferred_element_type=f32)
                        for hd in heads(g)]

        def b_softmax():
            ps, rs = [], []
            for sc in Bs['sc']:
                sc = jnp.where(valid, sc, fill)
                m = jnp.max(sc, axis=-1, keepdims=True)
                e = jnp.exp2((sc - m) * cB)
                l = jnp.sum(e, axis=-1, keepdims=True)
                r0 = pl.reciprocal(l, approx=True)
                r0 = r0 * (2.0 - l * r0)
                r0 = r0 * (2.0 - l * r0)
                ps.append(e.astype(bf16))
                rs.append(r0)
            Bs['p'], Bs['r'] = ps, rs

        def b_pv(g):
            Bs['oh'] = [jnp.dot(Bs['p'][i], v_ref[:, hd * DHB:(hd + 1) * DHB], preferred_element_type=f32)
                        for i, hd in enumerate(heads(g))]

        def b_norm(g):
            for i, hd in enumerate(heads(g)):
                o_ref[:, hd * DHB:(hd + 1) * DHB] = (Bs['oh'][i] * Bs['r'][i]).astype(bf16)

        def b_wo(g):
            cs = slice(g * GW, (g + 1) * GW)
            if parity == 0:
                lhs = jnp.concatenate([oe_ref[16:32, cs],
                                       jnp.where(lowhalf, oe_ref[32:48, cs], oe_ref[0:16, cs])], axis=0)
            else:
                lhs = jnp.concatenate([oo_ref[0:32, cs],
                                       jnp.where(lowhalf, oe_ref[0:16, cs], oo_ref[32:48, cs])], axis=0)
            part = jnp.dot(lhs, pltpu.bitcast(wo2_ref[g * GW // 2:(g + 1) * GW // 2, :], bf16),
                           preferred_element_type=f32)
            Bs['acc'] = part if Bs['acc'] is None else Bs['acc'] + part

        a_init()
        if parity == 0:
            h48_ref[0:32, :] = x_ref[pl.ds(base, 32), :]
            h48_ref[40:48, :] = x_ref[pl.ds(base + 32, 8), :]
            Bs['hh'] = h48_ref[...]
        else:
            h32_ref[0:16, :] = x_ref[pl.ds(base + 48, 16), :]
            h32_ref[24:32, :] = x_ref[pl.ds(base + 40, 8), :]
            Bs['hh'] = h32_ref[...]
        NP = GW // PW
        n_mid_slots = 3 * NG * NP
        n_mid = NTILES - A_HEAD - 3 * A_TAIL
        slot = [0, 0]

        def proj_all(g, which):
            for piece in range(NP):
                proj1(g, which, piece)
                slot[0] += 1
                tgt = (n_mid * slot[0]) // n_mid_slots
                a_tiles(tgt - slot[1])
                slot[1] = tgt

        a_tiles(A_HEAD)
        proj_all(0, 'q'); proj_all(0, 'k'); proj_all(0, 'v')
        prep_next()
        for g in range(NG):
            last = g + 1 == NG
            b_scores(g)
            if not last:
                proj_all(g + 1, 'q')
            else:
                a_tiles(A_TAIL)
            b_softmax()
            b_pv(g)
            if not last:
                proj_all(g + 1, 'k')
            else:
                a_tiles(A_TAIL)
            b_norm(g)
            b_wo(g)
            if not last:
                proj_all(g + 1, 'v')
            else:
                a_tiles(A_TAIL)
        outb = Bs['acc'].astype(bf16)
        if parity == 0:
            b_ref[pl.ds(base + 16, 16), :] = outb[0:16, :]
            h32_ref[16:24, :] = outb[16:24, :]
            b_ref[pl.ds(base + 8, 8), :] = outb[24:32, :]
        else:
            b_ref[pl.ds(base + 48, 16), :] = outb[0:16, :]
            h48_ref[32:40, :] = outb[16:24, :]
            b_ref[pl.ds(base + 40, 8), :] = outb[24:32, :]
            b_ref[pl.ds(base, 8), :] = outb[32:40, :]
            b_ref[pl.ds(base + 32, 8), :] = outb[40:48, :]
        a_final()

    def body(t, carry):
        base = pl.multiple_of(t * (2 * SEG), 2 * SEG)
        t_next = jnp.minimum(t + 1, HA - 1)
        half_step(0, base, make_a_unit(t, 0), lambda: build_qm(t, 1))
        half_step(1, base, make_a_unit(t, 1), lambda: build_qm(t_next, 0))
        return carry

    build_qm(0, 0)
    jax.lax.fori_loop(0, S // (2 * SEG), body, 0)

    oa = oT_ref[...].T.astype(bf16)
    cp_awo.wait()
    a = jnp.dot(oa, awo_ref[...], preferred_element_type=f32).astype(bf16).astype(f32)
    logit = jnp.sum(x_ref[...].astype(f32) * gw_ref[...].astype(f32), axis=-1, keepdims=True)
    gate = 1.0 / (1.0 + jnp.exp(-logit))
    out_ref[...] = (gate * a + (1.0 - gate) * b_ref[...].astype(f32)).astype(bf16)


TQ, TW, KB, HG, LA = 1024, 128, 128, 8, 12
PW, A_HEAD, A_TAIL = 128, 8, 8


@functools.partial(jax.jit, static_argnames=("B_seg_len",))
def pallas_gated_mix__mha_block__memory_aug_recurrent_mem_tr__prompt_kernel(
    A_x: jax.Array,
    A_wqkv: jax.Array,
    A_wo: jax.Array,
    B_x: jax.Array,
    B_mem0: jax.Array,
    B_Wq: jax.Array,
    B_Wk: jax.Array,
    B_Wv: jax.Array,
    B_Wo: jax.Array,
    B_seg_len: int,
    gate_w: jax.Array,
):
    Bsz, S, D = A_x.shape
    HA, DHA = 32, D // 32
    HB, DHB = B_Wq.shape[1], B_Wq.shape[2]
    M = B_mem0.shape[1]
    SEG = int(B_seg_len)
    assert Bsz == 1 and DHA == 16 and DHB == 128 and M == 8 and SEG == 32
    assert S == 2 * TQ and HA * (S // TQ) == S // SEG and HB % HG == 0
    R = 48

    x = A_x.reshape(S, D)
    mem0 = B_mem0.reshape(M, D)
    wq = B_Wq.reshape(D * HB, DHB)
    wk = B_Wk.reshape(D * HB, DHB)
    wv = B_Wv.reshape(D * HB, DHB)
    wo = B_Wo.reshape(HB * DHB, D)
    gw = gate_w.reshape(1, D)

    kernel = functools.partial(_kernel, S=S, D=D, HA=HA, DHA=DHA, HB=HB, DHB=DHB, SEG=SEG,
                               TQ=TQ, TW=TW, KB=KB, HG=HG, LA=LA, PW=PW, A_HEAD=A_HEAD, A_TAIL=A_TAIL)
    hbm = pl.BlockSpec(memory_space=pl.ANY)
    vmem = pl.BlockSpec(memory_space=pltpu.VMEM)
    out = pl.pallas_call(
        kernel,
        out_shape=jax.ShapeDtypeStruct((S, D), bf16),
        in_specs=[hbm, hbm, hbm, vmem, hbm, hbm, hbm, hbm, vmem],
        scratch_shapes=[
            pltpu.VMEM((S, D), bf16),
            pltpu.VMEM((D, 3 * D), bf16),
            pltpu.VMEM((D, D), bf16),
            pltpu.VMEM((D * HB, DHB), bf16),
            pltpu.VMEM((D * HB, DHB), bf16),
            pltpu.VMEM((D * HB, DHB), bf16),
            pltpu.VMEM((HB * DHB, D), bf16),
            pltpu.SemaphoreType.DMA((7,)),
            pltpu.VMEM((S, D), bf16),
            pltpu.VMEM((D, S), bf16),
            pltpu.VMEM((D, S), bf16),
            pltpu.VMEM((D, S), f32),
            pltpu.VMEM((64, TQ), u32),
            pltpu.VMEM((64, TQ), u32),
            pltpu.VMEM((S, D), bf16),
            pltpu.VMEM((48, D), bf16),
            pltpu.VMEM((32, D), bf16),
            pltpu.VMEM((R, HB * DHB), bf16),
            pltpu.VMEM((R, HB * DHB), bf16),
            pltpu.VMEM((R, HB * DHB), bf16),
            pltpu.VMEM((R, HB * DHB), bf16),
            pltpu.VMEM((R, HB * DHB), bf16),
            pltpu.VMEM((D // 2, HB * DHB), u32),
            pltpu.VMEM((D // 2, HB * DHB), u32),
            pltpu.VMEM((D // 2, HB * DHB), u32),
            pltpu.VMEM((HB * DHB // 2, D), u32),
        ],
        compiler_params=pltpu.CompilerParams(vmem_limit_bytes=100 * 1024 * 1024),
    )(x, A_wqkv, A_wo, mem0, wq, wk, wv, wo, gw)
    return out.reshape(Bsz, S, D)
```

```python
import functools

import jax
import jax.numpy as jnp
import jax.experimental.pallas as pl
import jax.experimental.pallas.tpu as pltpu

bf16 = jnp.bfloat16
f32 = jnp.float32
u32 = jnp.uint32
LOG2E = 1.4426950408889634


def _pack(v):
    return pltpu.bitcast(v, u32)


def _unpack(w):
    return pltpu.bitcast(w, bf16)


def _kernel(x_hbm, awqkv_hbm, awo_hbm, mem0_ref, wq_hbm, wk_hbm, wv_hbm, wo_hbm, gw_ref,
            out_ref,
            x_ref, awqkv_ref, awo_ref, wq_ref, wk_ref, wv_ref, wo_ref, sems,
            ka_ref, qT_ref, vT_ref, oT_ref, qm32e_ref, qm32o_ref,
            b_ref, h48_ref, h32_ref, q_ref, k_ref, v_ref, oe_ref, oo_ref,
            wq2_ref, wk2_ref, wv2_ref, wo2_ref,
            *, S, D, HA, DHA, HB, DHB, SEG, TQ, TW, KB, HG, LA, PW, A_HEAD, A_TAIL):
    NG = HB // HG
    GW = HG * DHB
    NK = S // KB
    NT = TQ // TW
    NTILES = NK * NT
    R = 48
    M = 8

    copies = [pltpu.make_async_copy(src, dst, sems.at[i]) for i, (src, dst) in enumerate([
        (x_hbm, x_ref), (awqkv_hbm, awqkv_ref), (wq_hbm, wq_ref), (wk_hbm, wk_ref),
        (wv_hbm, wv_ref), (wo_hbm, wo_ref), (awo_hbm, awo_ref)])]
    cp_x, cp_wqkv, cp_wq, cp_wk, cp_wv, cp_wo, cp_awo = copies
    cp_x.start()
    cp_wqkv.start()
    cp_x.wait()
    cp_wqkv.wait()
    for cp in (cp_wq, cp_wk, cp_wv, cp_wo, cp_awo):
        cp.start()

    def repack(raw_ref, dst_ref):
        raw32 = raw_ref.bitcast(u32)
        for j in range(HB // 2):
            for i0 in range(0, D // 2, 64):
                ev = raw32[pl.ds((2 * i0) * (HB // 2) + j, 64, stride=HB), :]
                od = raw32[pl.ds((2 * i0 + 1) * (HB // 2) + j, 64, stride=HB), :]
                dst_ref[i0:i0 + 64, (2 * j) * DHB:(2 * j + 1) * DHB] = (ev & jnp.uint32(0xFFFF)) | (od << 16)
                dst_ref[i0:i0 + 64, (2 * j + 1) * DHB:(2 * j + 2) * DHB] = (ev >> 16) | (od & jnp.uint32(0xFFFF0000))

    x = x_ref[...]
    qa = jnp.dot(x, awqkv_ref[:, 0:D], preferred_element_type=f32).astype(bf16)
    cp_wq.wait()
    repack(wq_ref, wq2_ref)
    ka_ref[...] = pltpu.bitcast(jnp.dot(x, awqkv_ref[:, D:2 * D], preferred_element_type=f32).astype(bf16), u32)
    cp_wk.wait()
    repack(wk_ref, wk2_ref)
    va = jnp.dot(x, awqkv_ref[:, 2 * D:3 * D], preferred_element_type=f32).astype(bf16)
    qT_ref[...] = (qa.astype(f32) * (DHA ** -0.5)).T.astype(bf16)
    cp_wv.wait()
    repack(wv_ref, wv2_ref)
    vT_ref[...] = pltpu.bitcast(va.astype(f32).T.astype(bf16), u32)
    cp_wo.wait()
    for c0 in range(0, HB * DHB, 512):
        wo2_ref[c0 // 2:c0 // 2 + 256, :] = pltpu.bitcast(wo_ref[c0:c0 + 512, :], u32)
    rowg = jax.lax.broadcasted_iota(jnp.int32, (128, TQ), 0) // DHA

    h48_ref[16:20, :] = _pack(mem0_ref[...])
    scale = DHB ** -0.5
    cB = scale * LOG2E

    def classify(idx, parity):
        if parity == 0:
            return idx, (idx >= 32) & (idx < 40), idx < 40
        t = jnp.where(idx < 16, idx + 16, jnp.where(idx >= 40, idx - 40, idx - 16))
        return t, (idx >= 16) & (idx < 24), (idx < 32) | (idx >= 40)

    ri = jax.lax.broadcasted_iota(jnp.int32, (R, R), 0)
    ci = jax.lax.broadcasted_iota(jnp.int32, (R, R), 1)
    valids, fills = [], []
    for parity in (0, 1):
        ti, mi, oki = classify(ri, parity)
        tj, mj, okj = classify(ci, parity)
        valids.append(okj & (mj | mi | (~oki) | (tj <= ti)))
        fills.append(jnp.where(okj, -1e9 / scale, -3e38).astype(f32))
    lowhalf = jax.lax.broadcasted_iota(jnp.int32, (8, GW), 0) < 4

    def build_qm(h, qb):
        g_ = h // (128 // DHA)
        r_ = h % (128 // DHA)
        gstart = pl.multiple_of(g_ * 128, 128)
        qg = qT_ref[pl.ds(gstart, 128), qb * TQ:(qb + 1) * TQ]
        qm32_ref = qm32e_ref if qb == 0 else qm32o_ref
        qm32_ref[...] = pltpu.bitcast(jnp.where(rowg == r_, qg.astype(f32), 0.0).astype(bf16), u32)

    def make_a_unit(h, qb):
        g_ = h // (128 // DHA)
        qstart = qb * TQ
        gstart = pl.multiple_of(g_ * 128, 128)
        hstart = pl.multiple_of(h * DHA, DHA)
        hstart2 = pl.multiple_of(h * (DHA // 2), DHA // 2)
        qm32_ref = qm32e_ref if qb == 0 else qm32o_ref
        A = {'issued': 0, 'done': 0, 'S': {}, 'm': [None] * NT, 'l': [None] * NT, 'acc': [None] * NT}

        def issue():
            j = A['issued']
            kb, qt = divmod(j, NT)
            A['S'][j] = jnp.dot(pltpu.bitcast(ka_ref[kb * KB // 2:(kb + 1) * KB // 2, pl.ds(gstart, 128)], bf16),
                                pltpu.bitcast(qm32_ref[:, qt * TW:(qt + 1) * TW], bf16),
                                preferred_element_type=f32)
            A['issued'] = j + 1

        def a_init():
            for _ in range(LA):
                issue()

        def a_tile():
            j = A['done']
            kb, qt = divmod(j, NT)
            if A['issued'] < NTILES:
                issue()
            s = A['S'].pop(j)
            bm = jnp.max(s, axis=0, keepdims=True)
            vT = pltpu.bitcast(vT_ref[pl.ds(hstart2, DHA // 2), kb * KB:(kb + 1) * KB], bf16)
            if kb == 0:
                m_new = bm
                e = jnp.exp(s - m_new)
                A['l'][qt] = jnp.sum(e, axis=0, keepdims=True)
                A['acc'][qt] = jnp.dot(vT, e.astype(bf16), preferred_element_type=f32)
            else:
                m_new = jnp.maximum(A['m'][qt], bm)
                alpha = jnp.exp(A['m'][qt] - m_new)
                e = jnp.exp(s - m_new)
                A['l'][qt] = alpha * A['l'][qt] + jnp.sum(e, axis=0, keepdims=True)
                A['acc'][qt] = alpha * A['acc'][qt] + jnp.dot(vT, e.astype(bf16), preferred_element_type=f32)
            A['m'][qt] = m_new
            A['done'] = j + 1

        def a_tiles(n):
            for _ in range(n):
                if A['done'] < NTILES:
                    a_tile()

        def a_final():
            assert A['done'] == NTILES
            for qt in range(NT):
                oT_ref[pl.ds(hstart, DHA), qstart + qt * TW:qstart + (qt + 1) * TW] = A['acc'][qt] / A['l'][qt]

        return a_init, a_tiles, a_final

    def half_step(parity, base, a_unit, prep_next):
        a_init, a_tiles, a_final = a_unit
        valid, fill = valids[parity], fills[parity]
        o_ref = oe_ref if parity == 0 else oo_ref
        RP = 48 if parity == 0 else 32
        Bs = {'acc': None}

        def proj1(g, which, piece):
            w_ref, dst_ref = {'q': (wq2_ref, q_ref), 'k': (wk2_ref, k_ref), 'v': (wv2_ref, v_ref)}[which]
            cs = slice(g * GW + piece * PW, g * GW + (piece + 1) * PW)
            dst_ref[0:RP // 2, cs] = _pack(jnp.dot(Bs['hh'], _unpack(w_ref[:, cs]),
                                                   preferred_element_type=f32).astype(bf16))

        def heads(g):
            return range(g * HG, (g + 1) * HG)

        def b_scores(g):
            Bs['sc'] = [jax.lax.dot_general(_unpack(q_ref[:, hd * DHB:(hd + 1) * DHB]), _unpack(k_ref[:, hd * DHB:(hd + 1) * DHB]),
                                            (((1,), (1,)), ((), ())), preferred_element_type=f32)
                        for hd in heads(g)]

        def b_softmax():
            ps, rs = [], []
            for sc in Bs['sc']:
                sc = jnp.where(valid, sc, fill)
                m = jnp.max(sc, axis=-1, keepdims=True)
                e = jnp.exp2((sc - m) * cB)
                l = jnp.sum(e, axis=-1, keepdims=True)
                r0 = pl.reciprocal(l, approx=True)
                r0 = r0 * (2.0 - l * r0)
                r0 = r0 * (2.0 - l * r0)
                ps.append(e.astype(bf16))
                rs.append(r0)
            Bs['p'], Bs['r'] = ps, rs

        def b_pv(g):
            Bs['oh'] = [jnp.dot(Bs['p'][i], _unpack(v_ref[:, hd * DHB:(hd + 1) * DHB]), preferred_element_type=f32)
                        for i, hd in enumerate(heads(g))]

        def b_norm(g):
            for i, hd in enumerate(heads(g)):
                o_ref[:, hd * DHB:(hd + 1) * DHB] = _pack((Bs['oh'][i] * Bs['r'][i]).astype(bf16))

        def b_wo(g):
            cs = slice(g * GW, (g + 1) * GW)
            if parity == 0:
                lhs = jnp.concatenate([oe_ref[8:16, cs],
                                       jnp.where(lowhalf, oe_ref[16:24, cs], oe_ref[0:8, cs])], axis=0)
            else:
                lhs = jnp.concatenate([oo_ref[0:16, cs],
                                       jnp.where(lowhalf, oe_ref[0:8, cs], oo_ref[16:24, cs])], axis=0)
            part = jnp.dot(_unpack(lhs), _unpack(wo2_ref[g * GW // 2:(g + 1) * GW // 2, :]),
                           preferred_element_type=f32)
            Bs['acc'] = part if Bs['acc'] is None else Bs['acc'] + part

        a_init()
        if parity == 0:
            h48_ref[0:16, :] = _pack(x_ref[pl.ds(base, 32), :])
            h48_ref[20:24, :] = _pack(x_ref[pl.ds(base + 32, 8), :])
            Bs['hh'] = _unpack(h48_ref[...])
        else:
            h32_ref[0:8, :] = _pack(x_ref[pl.ds(base + 48, 16), :])
            h32_ref[12:16, :] = _pack(x_ref[pl.ds(base + 40, 8), :])
            Bs['hh'] = _unpack(h32_ref[...])
        NP = GW // PW
        n_mid_slots = 3 * NG * NP
        n_mid = NTILES - A_HEAD - 3 * A_TAIL
        slot = [0, 0]

        def proj_all(g, which):
            for piece in range(NP):
                proj1(g, which, piece)
                slot[0] += 1
                tgt = (n_mid * slot[0]) // n_mid_slots
                a_tiles(tgt - slot[1])
                slot[1] = tgt

        a_tiles(A_HEAD)
        proj_all(0, 'q'); proj_all(0, 'k'); proj_all(0, 'v')
        prep_next()
        for g in range(NG):
            last = g + 1 == NG
            b_scores(g)
            if not last:
                proj_all(g + 1, 'q')
            else:
                a_tiles(A_TAIL)
            b_softmax()
            b_pv(g)
            if not last:
                proj_all(g + 1, 'k')
            else:
                a_tiles(A_TAIL)
            b_norm(g)
            b_wo(g)
            if not last:
                proj_all(g + 1, 'v')
            else:
                a_tiles(A_TAIL)
        outb = Bs['acc'].astype(bf16)
        if parity == 0:
            b_ref[pl.ds(base + 16, 16), :] = outb[0:16, :]
            h32_ref[8:12, :] = _pack(outb[16:24, :])
            b_ref[pl.ds(base + 8, 8), :] = outb[24:32, :]
        else:
            b_ref[pl.ds(base + 48, 16), :] = outb[0:16, :]
            h48_ref[16:20, :] = _pack(outb[16:24, :])
            b_ref[pl.ds(base + 40, 8), :] = outb[24:32, :]
            b_ref[pl.ds(base, 8), :] = outb[32:40, :]
            b_ref[pl.ds(base + 32, 8), :] = outb[40:48, :]
        a_final()

    def body(t, carry):
        base = pl.multiple_of(t * (2 * SEG), 2 * SEG)
        t_next = jnp.minimum(t + 1, HA - 1)
        half_step(0, base, make_a_unit(t, 0), lambda: build_qm(t, 1))
        half_step(1, base, make_a_unit(t, 1), lambda: build_qm(t_next, 0))
        return carry

    build_qm(0, 0)
    jax.lax.fori_loop(0, S // (2 * SEG), body, 0)

    oa = oT_ref[...].T.astype(bf16)
    cp_awo.wait()
    a = jnp.dot(oa, awo_ref[...], preferred_element_type=f32).astype(bf16).astype(f32)
    logit = jnp.sum(x_ref[...].astype(f32) * gw_ref[...].astype(f32), axis=-1, keepdims=True)
    gate = 1.0 / (1.0 + jnp.exp(-logit))
    out_ref[...] = (gate * a + (1.0 - gate) * b_ref[...].astype(f32)).astype(bf16)


TQ, TW, KB, HG, LA = 1024, 128, 128, 8, 12
PW, A_HEAD, A_TAIL = 128, 8, 8


@functools.partial(jax.jit, static_argnames=("B_seg_len",))
def pallas_gated_mix__mha_block__memory_aug_recurrent_mem_tr__prompt_kernel(
    A_x: jax.Array,
    A_wqkv: jax.Array,
    A_wo: jax.Array,
    B_x: jax.Array,
    B_mem0: jax.Array,
    B_Wq: jax.Array,
    B_Wk: jax.Array,
    B_Wv: jax.Array,
    B_Wo: jax.Array,
    B_seg_len: int,
    gate_w: jax.Array,
):
    Bsz, S, D = A_x.shape
    HA, DHA = 32, D // 32
    HB, DHB = B_Wq.shape[1], B_Wq.shape[2]
    M = B_mem0.shape[1]
    SEG = int(B_seg_len)
    assert Bsz == 1 and DHA == 16 and DHB == 128 and M == 8 and SEG == 32
    assert S == 2 * TQ and HA * (S // TQ) == S // SEG and HB % HG == 0
    R = 48

    x = A_x.reshape(S, D)
    mem0 = B_mem0.reshape(M, D)
    wq = B_Wq.reshape(D * HB, DHB)
    wk = B_Wk.reshape(D * HB, DHB)
    wv = B_Wv.reshape(D * HB, DHB)
    wo = B_Wo.reshape(HB * DHB, D)
    gw = gate_w.reshape(1, D)

    kernel = functools.partial(_kernel, S=S, D=D, HA=HA, DHA=DHA, HB=HB, DHB=DHB, SEG=SEG,
                               TQ=TQ, TW=TW, KB=KB, HG=HG, LA=LA, PW=PW, A_HEAD=A_HEAD, A_TAIL=A_TAIL)
    hbm = pl.BlockSpec(memory_space=pl.ANY)
    vmem = pl.BlockSpec(memory_space=pltpu.VMEM)
    out = pl.pallas_call(
        kernel,
        out_shape=jax.ShapeDtypeStruct((S, D), bf16),
        in_specs=[hbm, hbm, hbm, vmem, hbm, hbm, hbm, hbm, vmem],
        scratch_shapes=[
            pltpu.VMEM((S, D), bf16),
            pltpu.VMEM((D, 3 * D), bf16),
            pltpu.VMEM((D, D), bf16),
            pltpu.VMEM((D * HB, DHB), bf16),
            pltpu.VMEM((D * HB, DHB), bf16),
            pltpu.VMEM((D * HB, DHB), bf16),
            pltpu.VMEM((HB * DHB, D), bf16),
            pltpu.SemaphoreType.DMA((7,)),
            pltpu.VMEM((S // 2, D), u32),
            pltpu.VMEM((D, S), bf16),
            pltpu.VMEM((D // 2, S), u32),
            pltpu.VMEM((D, S), f32),
            pltpu.VMEM((64, TQ), u32),
            pltpu.VMEM((64, TQ), u32),
            pltpu.VMEM((S, D), bf16),
            pltpu.VMEM((24, D), u32),
            pltpu.VMEM((16, D), u32),
            pltpu.VMEM((R // 2, HB * DHB), u32),
            pltpu.VMEM((R // 2, HB * DHB), u32),
            pltpu.VMEM((R // 2, HB * DHB), u32),
            pltpu.VMEM((R // 2, HB * DHB), u32),
            pltpu.VMEM((R // 2, HB * DHB), u32),
            pltpu.VMEM((D // 2, HB * DHB), u32),
            pltpu.VMEM((D // 2, HB * DHB), u32),
            pltpu.VMEM((D // 2, HB * DHB), u32),
            pltpu.VMEM((HB * DHB // 2, D), u32),
        ],
        compiler_params=pltpu.CompilerParams(vmem_limit_bytes=100 * 1024 * 1024),
    )(x, A_wqkv, A_wo, mem0, wq, wk, wv, wo, gw)
    return out.reshape(Bsz, S, D)
```

```python
import functools

import jax
import jax.numpy as jnp
import jax.experimental.pallas as pl
import jax.experimental.pallas.tpu as pltpu

bf16 = jnp.bfloat16
f32 = jnp.float32
u32 = jnp.uint32
LOG2E = 1.4426950408889634


def _pack(v):
    return pltpu.bitcast(v, u32)


def _unpack(w):
    return pltpu.bitcast(w, bf16)


def _kernel(x_hbm, awqkv_hbm, awo_hbm, mem0_ref, wq_hbm, wk_hbm, wv_hbm, wo_hbm, gw_ref,
            out_hbm,
            x_ref, awqkv_ref, awo_ref, wq_ref, wk_ref, wv_ref, wo_ref, sems, ob_ref, osems,
            ka_ref, qT_ref, vT_ref, oT_ref, qm32e_ref, qm32o_ref,
            b_ref, h48_ref, h32_ref, q_ref, k_ref, v_ref, oe_ref, oo_ref,
            wq2_ref, wk2_ref, wv2_ref, wo2_ref,
            *, S, D, HA, DHA, HB, DHB, SEG, TQ, TW, KB, HG, LA, PW, A_HEAD, A_TAIL, PVD):
    NG = HB // HG
    GW = HG * DHB
    NK = S // KB
    NT = TQ // TW
    NTILES = NK * NT
    R = 48
    M = 8

    copies = [pltpu.make_async_copy(src, dst, sems.at[i]) for i, (src, dst) in enumerate([
        (x_hbm, x_ref), (awqkv_hbm, awqkv_ref), (wq_hbm, wq_ref), (wk_hbm, wk_ref),
        (wv_hbm, wv_ref), (wo_hbm, wo_ref), (awo_hbm, awo_ref)])]
    cp_x, cp_wqkv, cp_wq, cp_wk, cp_wv, cp_wo, cp_awo = copies
    for cp in copies:
        cp.start()
    cp_x.wait()
    cp_wqkv.wait()

    sub8 = jax.lax.broadcasted_iota(jnp.int32, (8, 128), 0)

    def transpose8(X):
        X = list(X)
        for s in (1, 2, 4):
            keep = (sub8 & s) == 0
            for k in range(8):
                if k & s == 0:
                    a, b = X[k], X[k + s]
                    X[k] = jnp.where(keep, a, pltpu.roll(b, s, 0))
                    X[k + s] = jnp.where(keep, pltpu.roll(a, 8 - s, 0), b)
        return X

    def repack(raw_ref, dst_ref):
        HP = HB // 2
        raw32 = raw_ref.bitcast(u32)
        for b in range(D // 16):
            for c in range(HP // 8):
                los, his = [], []
                for k in range(8):
                    r0 = (16 * b + 2 * k) * HP + 8 * c
                    ev = raw32[r0:r0 + 8, :]
                    od = raw32[r0 + HP:r0 + HP + 8, :]
                    los.append((ev & jnp.uint32(0xFFFF)) | (od << 16))
                    his.append((ev >> 16) | (od & jnp.uint32(0xFFFF0000)))
                los, his = transpose8(los), transpose8(his)
                for j in range(8):
                    h = 2 * (8 * c + j)
                    dst_ref[8 * b:8 * b + 8, h * DHB:(h + 1) * DHB] = los[j]
                    dst_ref[8 * b:8 * b + 8, (h + 1) * DHB:(h + 2) * DHB] = his[j]

    x = x_ref[...]
    qa = jnp.dot(x, awqkv_ref[:, 0:D], preferred_element_type=f32).astype(bf16)
    cp_wq.wait()
    repack(wq_ref, wq2_ref)
    ka_ref[...] = pltpu.bitcast(jnp.dot(x, awqkv_ref[:, D:2 * D], preferred_element_type=f32).astype(bf16), u32)
    cp_wk.wait()
    repack(wk_ref, wk2_ref)
    va = jnp.dot(x, awqkv_ref[:, 2 * D:3 * D], preferred_element_type=f32).astype(bf16)
    qT_ref[...] = (qa.astype(f32) * (DHA ** -0.5)).T.astype(bf16)
    cp_wv.wait()
    repack(wv_ref, wv2_ref)
    vT_ref[...] = pltpu.bitcast(va.astype(f32).T.astype(bf16), u32)
    cp_wo.wait()
    for c0 in range(0, HB * DHB, 512):
        wo2_ref[c0 // 2:c0 // 2 + 256, :] = pltpu.bitcast(wo_ref[c0:c0 + 512, :], u32)
    rowg = jax.lax.broadcasted_iota(jnp.int32, (128, TQ), 0) // DHA

    h48_ref[16:20, :] = _pack(mem0_ref[...])
    scale = DHB ** -0.5
    cB = scale * LOG2E

    def classify(idx, parity):
        if parity == 0:
            return idx, (idx >= 32) & (idx < 40), idx < 40
        t = jnp.where(idx < 16, idx + 16, jnp.where(idx >= 40, idx - 40, idx - 16))
        return t, (idx >= 16) & (idx < 24), (idx < 32) | (idx >= 40)

    ri = jax.lax.broadcasted_iota(jnp.int32, (R, R), 0)
    ci = jax.lax.broadcasted_iota(jnp.int32, (R, R), 1)
    valids, fills = [], []
    for parity in (0, 1):
        ti, mi, oki = classify(ri, parity)
        tj, mj, okj = classify(ci, parity)
        valids.append(okj & (mj | mi | (~oki) | (tj <= ti)))
        fills.append(jnp.where(okj, -1e9 / scale, -3e38).astype(f32))
    lowhalf = jax.lax.broadcasted_iota(jnp.int32, (8, GW), 0) < 4

    def build_qm(h, qb):
        g_ = h // (128 // DHA)
        r_ = h % (128 // DHA)
        gstart = pl.multiple_of(g_ * 128, 128)
        qg = qT_ref[pl.ds(gstart, 128), qb * TQ:(qb + 1) * TQ]
        qm32_ref = qm32e_ref if qb == 0 else qm32o_ref
        qm32_ref[...] = pltpu.bitcast(jnp.where(rowg == r_, qg.astype(f32), 0.0).astype(bf16), u32)

    def make_a_unit(h, qb):
        g_ = h // (128 // DHA)
        qstart = qb * TQ
        gstart = pl.multiple_of(g_ * 128, 128)
        hstart = pl.multiple_of(h * DHA, DHA)
        hstart2 = pl.multiple_of(h * (DHA // 2), DHA // 2)
        qm32_ref = qm32e_ref if qb == 0 else qm32o_ref
        A = {'issued': 0, 'done': 0, 'S': {}, 'P': {}, 'm': [None] * NT, 'l': [None] * NT, 'acc': [None] * NT}

        def issue():
            j = A['issued']
            kb, qt = divmod(j, NT)
            A['S'][j] = jnp.dot(pltpu.bitcast(ka_ref[kb * KB // 2:(kb + 1) * KB // 2, pl.ds(gstart, 128)], bf16),
                                pltpu.bitcast(qm32_ref[:, qt * TW:(qt + 1) * TW], bf16),
                                preferred_element_type=f32)
            A['issued'] = j + 1

        def a_init():
            for _ in range(LA):
                issue()

        def a_pv(j):
            kb, qt = divmod(j, NT)
            p, alpha = A['P'].pop(j)
            vT = _unpack(vT_ref[pl.ds(hstart2, DHA // 2), kb * KB:(kb + 1) * KB])
            part = jnp.dot(vT, p, preferred_element_type=f32)
            A['acc'][qt] = part if kb == 0 else alpha * A['acc'][qt] + part

        def a_tile():
            j = A['done']
            kb, qt = divmod(j, NT)
            if A['issued'] < NTILES:
                issue()
            s = A['S'].pop(j)
            bm = jnp.max(s, axis=0, keepdims=True)
            if kb == 0:
                m_new, alpha = bm, None
                e = jnp.exp(s - m_new)
                A['l'][qt] = jnp.sum(e, axis=0, keepdims=True)
            else:
                m_new = jnp.maximum(A['m'][qt], bm)
                alpha = jnp.exp(A['m'][qt] - m_new)
                e = jnp.exp(s - m_new)
                A['l'][qt] = alpha * A['l'][qt] + jnp.sum(e, axis=0, keepdims=True)
            A['m'][qt] = m_new
            A['P'][j] = (e.astype(bf16), alpha)
            if j >= PVD:
                a_pv(j - PVD)
            A['done'] = j + 1

        def a_tiles(n):
            for _ in range(n):
                if A['done'] < NTILES:
                    a_tile()

        def a_final():
            assert A['done'] == NTILES
            for j in range(NTILES - PVD, NTILES):
                a_pv(j)
            for qt in range(NT):
                oT_ref[pl.ds(hstart, DHA), qstart + qt * TW:qstart + (qt + 1) * TW] = A['acc'][qt] / A['l'][qt]

        return a_init, a_tiles, a_final

    def half_step(parity, base, a_unit, prep_next):
        a_init, a_tiles, a_final = a_unit
        valid, fill = valids[parity], fills[parity]
        o_ref = oe_ref if parity == 0 else oo_ref
        RP = 48 if parity == 0 else 32
        Bs = {'acc': None}

        def proj1(g, which, piece):
            w_ref, dst_ref = {'q': (wq2_ref, q_ref), 'k': (wk2_ref, k_ref), 'v': (wv2_ref, v_ref)}[which]
            cs = slice(g * GW + piece * PW, g * GW + (piece + 1) * PW)
            dst_ref[0:RP // 2, cs] = _pack(jnp.dot(Bs['hh'], _unpack(w_ref[:, cs]),
                                                   preferred_element_type=f32).astype(bf16))

        def heads(g):
            return range(g * HG, (g + 1) * HG)

        def b_scores(g):
            Bs['sc'] = [jax.lax.dot_general(_unpack(q_ref[:, hd * DHB:(hd + 1) * DHB]), _unpack(k_ref[:, hd * DHB:(hd + 1) * DHB]),
                                            (((1,), (1,)), ((), ())), preferred_element_type=f32)
                        for hd in heads(g)]

        def b_softmax():
            ps, rs = [], []
            for sc in Bs['sc']:
                sc = jnp.where(valid, sc, fill)
                m = jnp.max(sc, axis=-1, keepdims=True)
                e = jnp.exp2((sc - m) * cB)
                l = jnp.sum(e, axis=-1, keepdims=True)
                r0 = pl.reciprocal(l, approx=True)
                r0 = r0 * (2.0 - l * r0)
                r0 = r0 * (2.0 - l * r0)
                ps.append(e.astype(bf16))
                rs.append(r0)
            Bs['p'], Bs['r'] = ps, rs

        def b_pv(g):
            Bs['oh'] = [jnp.dot(Bs['p'][i], _unpack(v_ref[:, hd * DHB:(hd + 1) * DHB]), preferred_element_type=f32)
                        for i, hd in enumerate(heads(g))]

        def b_norm(g):
            for i, hd in enumerate(heads(g)):
                o_ref[:, hd * DHB:(hd + 1) * DHB] = _pack((Bs['oh'][i] * Bs['r'][i]).astype(bf16))

        def b_wo(g):
            cs = slice(g * GW, (g + 1) * GW)
            if parity == 0:
                lhs = jnp.concatenate([oe_ref[8:16, cs],
                                       jnp.where(lowhalf, oe_ref[16:24, cs], oe_ref[0:8, cs])], axis=0)
            else:
                lhs = jnp.concatenate([oo_ref[0:16, cs],
                                       jnp.where(lowhalf, oe_ref[0:8, cs], oo_ref[16:24, cs])], axis=0)
            part = jnp.dot(_unpack(lhs), _unpack(wo2_ref[g * GW // 2:(g + 1) * GW // 2, :]),
                           preferred_element_type=f32)
            Bs['acc'] = part if Bs['acc'] is None else Bs['acc'] + part

        a_init()
        if parity == 0:
            h48_ref[0:16, :] = _pack(x_ref[pl.ds(base, 32), :])
            h48_ref[20:24, :] = _pack(x_ref[pl.ds(base + 32, 8), :])
            Bs['hh'] = _unpack(h48_ref[...])
        else:
            h32_ref[0:8, :] = _pack(x_ref[pl.ds(base + 48, 16), :])
            h32_ref[12:16, :] = _pack(x_ref[pl.ds(base + 40, 8), :])
            Bs['hh'] = _unpack(h32_ref[...])
        NP = GW // PW
        n_mid_slots = 3 * NG * NP
        n_mid = NTILES - A_HEAD - 3 * A_TAIL
        slot = [0, 0]

        def proj_all(g, which):
            for piece in range(NP):
                proj1(g, which, piece)
                slot[0] += 1
                tgt = (n_mid * slot[0]) // n_mid_slots
                a_tiles(tgt - slot[1])
                slot[1] = tgt

        a_tiles(A_HEAD)
        proj_all(0, 'q'); proj_all(0, 'k'); proj_all(0, 'v')
        prep_next()
        for g in range(NG):
            last = g + 1 == NG
            b_scores(g)
            if not last:
                proj_all(g + 1, 'q')
            else:
                a_tiles(A_TAIL)
            b_softmax()
            b_pv(g)
            if not last:
                proj_all(g + 1, 'k')
            else:
                a_tiles(A_TAIL)
            b_norm(g)
            b_wo(g)
            if not last:
                proj_all(g + 1, 'v')
            else:
                a_tiles(A_TAIL)
        outb = Bs['acc'].astype(bf16)
        if parity == 0:
            b_ref[pl.ds(base + 16, 16), :] = outb[0:16, :]
            h32_ref[8:12, :] = _pack(outb[16:24, :])
            b_ref[pl.ds(base + 8, 8), :] = outb[24:32, :]
        else:
            b_ref[pl.ds(base + 48, 16), :] = outb[0:16, :]
            h48_ref[16:20, :] = _pack(outb[16:24, :])
            b_ref[pl.ds(base + 40, 8), :] = outb[24:32, :]
            b_ref[pl.ds(base, 8), :] = outb[32:40, :]
            b_ref[pl.ds(base + 32, 8), :] = outb[40:48, :]
        a_final()

    def body(t, carry):
        base = pl.multiple_of(t * (2 * SEG), 2 * SEG)
        t_next = jnp.minimum(t + 1, HA - 1)
        half_step(0, base, make_a_unit(t, 0), lambda: build_qm(t, 1))
        half_step(1, base, make_a_unit(t, 1), lambda: build_qm(t_next, 0))
        return carry

    build_qm(0, 0)
    jax.lax.fori_loop(0, S // (2 * SEG), body, 0)

    cp_awo.wait()
    awo = awo_ref[...]
    gw = gw_ref[...].astype(f32)
    outs = []
    for r in range(S // 128):
        rows = slice(r * 128, (r + 1) * 128)
        oa = oT_ref[:, rows].T.astype(bf16)
        a = jnp.dot(oa, awo, preferred_element_type=f32).astype(bf16).astype(f32)
        logit = jnp.sum(x_ref[rows, :].astype(f32) * gw, axis=-1, keepdims=True)
        gate = 1.0 / (1.0 + jnp.exp(-logit))
        ob_ref[rows, :] = (gate * a + (1.0 - gate) * b_ref[rows, :].astype(f32)).astype(bf16)
        cp = pltpu.make_async_copy(ob_ref.at[rows, :], out_hbm.at[rows, :], osems.at[r])
        cp.start()
        outs.append(cp)
    for cp in outs:
        cp.wait()


TQ, TW, KB, HG, LA = 1024, 128, 128, 8, 12
PVD = 0
PW, A_HEAD, A_TAIL = 128, 8, 8


@functools.partial(jax.jit, static_argnames=("B_seg_len",))
def pallas_gated_mix__mha_block__memory_aug_recurrent_mem_tr__prompt_kernel(
    A_x: jax.Array,
    A_wqkv: jax.Array,
    A_wo: jax.Array,
    B_x: jax.Array,
    B_mem0: jax.Array,
    B_Wq: jax.Array,
    B_Wk: jax.Array,
    B_Wv: jax.Array,
    B_Wo: jax.Array,
    B_seg_len: int,
    gate_w: jax.Array,
):
    Bsz, S, D = A_x.shape
    HA, DHA = 32, D // 32
    HB, DHB = B_Wq.shape[1], B_Wq.shape[2]
    M = B_mem0.shape[1]
    SEG = int(B_seg_len)
    assert Bsz == 1 and DHA == 16 and DHB == 128 and M == 8 and SEG == 32
    assert S == 2 * TQ and HA * (S // TQ) == S // SEG and HB % HG == 0
    R = 48

    x = A_x.reshape(S, D)
    mem0 = B_mem0.reshape(M, D)
    wq = B_Wq.reshape(D * HB, DHB)
    wk = B_Wk.reshape(D * HB, DHB)
    wv = B_Wv.reshape(D * HB, DHB)
    wo = B_Wo.reshape(HB * DHB, D)
    gw = gate_w.reshape(1, D)

    kernel = functools.partial(_kernel, S=S, D=D, HA=HA, DHA=DHA, HB=HB, DHB=DHB, SEG=SEG,
                               TQ=TQ, TW=TW, KB=KB, HG=HG, LA=LA, PW=PW, A_HEAD=A_HEAD, A_TAIL=A_TAIL, PVD=PVD)
    hbm = pl.BlockSpec(memory_space=pl.ANY)
    vmem = pl.BlockSpec(memory_space=pltpu.VMEM)
    out = pl.pallas_call(
        kernel,
        out_shape=jax.ShapeDtypeStruct((S, D), bf16),
        in_specs=[hbm, hbm, hbm, vmem, hbm, hbm, hbm, hbm, vmem],
        out_specs=hbm,
        scratch_shapes=[
            pltpu.VMEM((S, D), bf16),
            pltpu.VMEM((D, 3 * D), bf16),
            pltpu.VMEM((D, D), bf16),
            pltpu.VMEM((D * HB, DHB), bf16),
            pltpu.VMEM((D * HB, DHB), bf16),
            pltpu.VMEM((D * HB, DHB), bf16),
            pltpu.VMEM((HB * DHB, D), bf16),
            pltpu.SemaphoreType.DMA((7,)),
            pltpu.VMEM((S, D), bf16),
            pltpu.SemaphoreType.DMA((S // 128,)),
            pltpu.VMEM((S // 2, D), u32),
            pltpu.VMEM((D, S), bf16),
            pltpu.VMEM((D // 2, S), u32),
            pltpu.VMEM((D, S), f32),
            pltpu.VMEM((64, TQ), u32),
            pltpu.VMEM((64, TQ), u32),
            pltpu.VMEM((S, D), bf16),
            pltpu.VMEM((24, D), u32),
            pltpu.VMEM((16, D), u32),
            pltpu.VMEM((R // 2, HB * DHB), u32),
            pltpu.VMEM((R // 2, HB * DHB), u32),
            pltpu.VMEM((R // 2, HB * DHB), u32),
            pltpu.VMEM((R // 2, HB * DHB), u32),
            pltpu.VMEM((R // 2, HB * DHB), u32),
            pltpu.VMEM((D // 2, HB * DHB), u32),
            pltpu.VMEM((D // 2, HB * DHB), u32),
            pltpu.VMEM((D // 2, HB * DHB), u32),
            pltpu.VMEM((HB * DHB // 2, D), u32),
        ],
        compiler_params=pltpu.CompilerParams(vmem_limit_bytes=100 * 1024 * 1024),
    )(x, A_wqkv, A_wo, mem0, wq, wk, wv, wo, gw)
    return out.reshape(Bsz, S, D)
```

```python
import functools

import jax
import jax.numpy as jnp
import jax.experimental.pallas as pl
import jax.experimental.pallas.tpu as pltpu

bf16 = jnp.bfloat16
f32 = jnp.float32
u32 = jnp.uint32
LOG2E = 1.4426950408889634


def _pack(v):
    return pltpu.bitcast(v, u32)


def _unpack(w):
    return pltpu.bitcast(w, bf16)


def _kernel(x_hbm, awqkv_hbm, awo_hbm, mem0_ref, wq_hbm, wk_hbm, wv_hbm, wo_hbm, gw_ref,
            out_hbm,
            x_ref, awqkv_ref, awo_ref, wq_ref, wk_ref, wv_ref, wo_ref, sems, ob_ref, osems,
            ka_ref, qT_ref, vT_ref, oT_ref, qm32e_ref, qm32o_ref,
            b_ref, h48_ref, h32_ref, q_ref, k_ref, v_ref, oe_ref, oo_ref,
            wq2_ref, wk2_ref, wv2_ref, wo2_ref,
            *, S, D, HA, DHA, HB, DHB, SEG, TQ, TW, KB, HG, LA, PW, A_HEAD, A_TAIL, PVD):
    NG = HB // HG
    GW = HG * DHB
    NK = S // KB
    NT = TQ // TW
    NTILES = NK * NT
    R = 48

    copies = [pltpu.make_async_copy(src, dst, sems.at[i]) for i, (src, dst) in enumerate([
        (x_hbm, x_ref), (awqkv_hbm, awqkv_ref), (wq_hbm, wq_ref), (wk_hbm, wk_ref),
        (wv_hbm, wv_ref), (wo_hbm, wo_ref), (awo_hbm, awo_ref)])]
    cp_x, cp_wqkv, cp_wq, cp_wk, cp_wv, cp_wo, cp_awo = copies
    for cp in copies:
        cp.start()
    cp_x.wait()
    cp_wqkv.wait()

    sub8 = jax.lax.broadcasted_iota(jnp.int32, (8, 128), 0)

    def transpose8(X):
        X = list(X)
        for s in (1, 2, 4):
            keep = (sub8 & s) == 0
            for k in range(8):
                if k & s == 0:
                    a, b = X[k], X[k + s]
                    X[k] = jnp.where(keep, a, pltpu.roll(b, s, 0))
                    X[k + s] = jnp.where(keep, pltpu.roll(a, 8 - s, 0), b)
        return X

    def repack(raw_ref, dst_ref):
        HP = HB // 2

        def words(r):
            return _pack(raw_ref[2 * r:2 * r + 16, :])

        for b in range(D // 16):
            for c in range(HP // 8):
                los, his = [], []
                for k in range(8):
                    r0 = (16 * b + 2 * k) * HP + 8 * c
                    ev = words(r0)
                    od = words(r0 + HP)
                    los.append((ev & jnp.uint32(0xFFFF)) | (od << 16))
                    his.append((ev >> 16) | (od & jnp.uint32(0xFFFF0000)))
                los, his = transpose8(los), transpose8(his)
                for j in range(8):
                    h = 2 * (8 * c + j)
                    dst_ref[8 * b:8 * b + 8, h * DHB:(h + 1) * DHB] = los[j]
                    dst_ref[8 * b:8 * b + 8, (h + 1) * DHB:(h + 2) * DHB] = his[j]

    x = x_ref[...]
    qa = jnp.dot(x, awqkv_ref[:, 0:D], preferred_element_type=f32).astype(bf16)
    cp_wq.wait()
    repack(wq_ref, wq2_ref)
    ka_ref[...] = pltpu.bitcast(jnp.dot(x, awqkv_ref[:, D:2 * D], preferred_element_type=f32).astype(bf16), u32)
    cp_wk.wait()
    repack(wk_ref, wk2_ref)
    va = jnp.dot(x, awqkv_ref[:, 2 * D:3 * D], preferred_element_type=f32).astype(bf16)
    qT_ref[...] = (qa.astype(f32) * (DHA ** -0.5)).T.astype(bf16)
    cp_wv.wait()
    repack(wv_ref, wv2_ref)
    vT_ref[...] = pltpu.bitcast(va.astype(f32).T.astype(bf16), u32)
    cp_wo.wait()
    for c0 in range(0, HB * DHB, 512):
        wo2_ref[c0 // 2:c0 // 2 + 256, :] = pltpu.bitcast(wo_ref[c0:c0 + 512, :], u32)
    rowg = jax.lax.broadcasted_iota(jnp.int32, (128, TQ), 0) // DHA

    h48_ref[16:20, :] = _pack(mem0_ref[...])
    scale = DHB ** -0.5
    cB = scale * LOG2E

    def classify(idx, parity):
        if parity == 0:
            return idx, (idx >= 32) & (idx < 40), idx < 40
        t = jnp.where(idx < 16, idx + 16, jnp.where(idx >= 40, idx - 40, idx - 16))
        return t, (idx >= 16) & (idx < 24), (idx < 32) | (idx >= 40)

    ri = jax.lax.broadcasted_iota(jnp.int32, (R, R), 0)
    ci = jax.lax.broadcasted_iota(jnp.int32, (R, R), 1)
    valids, fills = [], []
    for parity in (0, 1):
        ti, mi, oki = classify(ri, parity)
        tj, mj, okj = classify(ci, parity)
        valids.append(okj & (mj | mi | (~oki) | (tj <= ti)))
        fills.append(jnp.where(okj, -1e9 / scale, -3e38).astype(f32))
    lowhalf = jax.lax.broadcasted_iota(jnp.int32, (8, GW), 0) < 4

    def build_qm(h, qb):
        g_ = h // (128 // DHA)
        r_ = h % (128 // DHA)
        gstart = pl.multiple_of(g_ * 128, 128)
        qg = qT_ref[pl.ds(gstart, 128), qb * TQ:(qb + 1) * TQ]
        qm32_ref = qm32e_ref if qb == 0 else qm32o_ref
        qm32_ref[...] = pltpu.bitcast(jnp.where(rowg == r_, qg.astype(f32), 0.0).astype(bf16), u32)

    def make_a_unit(h, qb):
        g_ = h // (128 // DHA)
        qstart = qb * TQ
        gstart = pl.multiple_of(g_ * 128, 128)
        hstart = pl.multiple_of(h * DHA, DHA)
        hstart2 = pl.multiple_of(h * (DHA // 2), DHA // 2)
        qm32_ref = qm32e_ref if qb == 0 else qm32o_ref
        A = {'issued': 0, 'done': 0, 'S': {}, 'P': {}, 'm': [None] * NT, 'l': [None] * NT, 'acc': [None] * NT}

        def issue():
            j = A['issued']
            kb, qt = divmod(j, NT)
            A['S'][j] = jnp.dot(pltpu.bitcast(ka_ref[kb * KB // 2:(kb + 1) * KB // 2, pl.ds(gstart, 128)], bf16),
                                pltpu.bitcast(qm32_ref[:, qt * TW:(qt + 1) * TW], bf16),
                                preferred_element_type=f32)
            A['issued'] = j + 1

        def a_init():
            for _ in range(LA):
                issue()

        def a_pv(j):
            kb, qt = divmod(j, NT)
            p, alpha = A['P'].pop(j)
            vT = _unpack(vT_ref[pl.ds(hstart2, DHA // 2), kb * KB:(kb + 1) * KB])
            part = jnp.dot(vT, p, preferred_element_type=f32)
            A['acc'][qt] = part if kb == 0 else alpha * A['acc'][qt] + part

        def a_tile():
            j = A['done']
            kb, qt = divmod(j, NT)
            if A['issued'] < NTILES:
                issue()
            s = A['S'].pop(j)
            bm = jnp.max(s, axis=0, keepdims=True)
            if kb == 0:
                m_new, alpha = bm, None
                e = jnp.exp(s - m_new)
                A['l'][qt] = jnp.sum(e, axis=0, keepdims=True)
            else:
                m_new = jnp.maximum(A['m'][qt], bm)
                alpha = jnp.exp(A['m'][qt] - m_new)
                e = jnp.exp(s - m_new)
                A['l'][qt] = alpha * A['l'][qt] + jnp.sum(e, axis=0, keepdims=True)
            A['m'][qt] = m_new
            A['P'][j] = (e.astype(bf16), alpha)
            if j >= PVD:
                a_pv(j - PVD)
            A['done'] = j + 1

        def a_tiles(n):
            for _ in range(n):
                if A['done'] < NTILES:
                    a_tile()

        def a_final():
            assert A['done'] == NTILES
            for j in range(NTILES - PVD, NTILES):
                a_pv(j)
            for qt in range(NT):
                oT_ref[pl.ds(hstart, DHA), qstart + qt * TW:qstart + (qt + 1) * TW] = A['acc'][qt] / A['l'][qt]

        return a_init, a_tiles, a_final

    def half_step(parity, base, a_unit, prep_next):
        a_init, a_tiles, a_final = a_unit
        valid, fill = valids[parity], fills[parity]
        o_ref = oe_ref if parity == 0 else oo_ref
        RP = 48 if parity == 0 else 32
        Bs = {'acc': None}

        def proj1(g, which, piece):
            w_ref, dst_ref = {'q': (wq2_ref, q_ref), 'k': (wk2_ref, k_ref), 'v': (wv2_ref, v_ref)}[which]
            cs = slice(g * GW + piece * PW, g * GW + (piece + 1) * PW)
            dst_ref[0:RP // 2, cs] = _pack(jnp.dot(Bs['hh'], _unpack(w_ref[:, cs]),
                                                   preferred_element_type=f32).astype(bf16))

        def heads(g):
            return range(g * HG, (g + 1) * HG)

        def b_scores(g):
            Bs['sc'] = [jax.lax.dot_general(_unpack(q_ref[:, hd * DHB:(hd + 1) * DHB]), _unpack(k_ref[:, hd * DHB:(hd + 1) * DHB]),
                                            (((1,), (1,)), ((), ())), preferred_element_type=f32)
                        for hd in heads(g)]

        def b_softmax():
            ps, rs = [], []
            for sc in Bs['sc']:
                sc = jnp.where(valid, sc, fill)
                m = jnp.max(sc, axis=-1, keepdims=True)
                e = jnp.exp2((sc - m) * cB)
                l = jnp.sum(e, axis=-1, keepdims=True)
                r0 = pl.reciprocal(l, approx=True)
                r0 = r0 * (2.0 - l * r0)
                r0 = r0 * (2.0 - l * r0)
                ps.append(e.astype(bf16))
                rs.append(r0)
            Bs['p'], Bs['r'] = ps, rs

        def b_pv(g):
            Bs['oh'] = [jnp.dot(Bs['p'][i], _unpack(v_ref[:, hd * DHB:(hd + 1) * DHB]), preferred_element_type=f32)
                        for i, hd in enumerate(heads(g))]

        def b_norm(g):
            for i, hd in enumerate(heads(g)):
                o_ref[:, hd * DHB:(hd + 1) * DHB] = _pack((Bs['oh'][i] * Bs['r'][i]).astype(bf16))

        def b_wo(g):
            cs = slice(g * GW, (g + 1) * GW)
            if parity == 0:
                lhs = jnp.concatenate([oe_ref[8:16, cs],
                                       jnp.where(lowhalf, oe_ref[16:24, cs], oe_ref[0:8, cs])], axis=0)
            else:
                lhs = jnp.concatenate([oo_ref[0:16, cs],
                                       jnp.where(lowhalf, oe_ref[0:8, cs], oo_ref[16:24, cs])], axis=0)
            part = jnp.dot(_unpack(lhs), _unpack(wo2_ref[g * GW // 2:(g + 1) * GW // 2, :]),
                           preferred_element_type=f32)
            Bs['acc'] = part if Bs['acc'] is None else Bs['acc'] + part

        a_init()
        if parity == 0:
            h48_ref[0:16, :] = _pack(x_ref[pl.ds(base, 32), :])
            h48_ref[20:24, :] = _pack(x_ref[pl.ds(base + 32, 8), :])
            Bs['hh'] = _unpack(h48_ref[...])
        else:
            h32_ref[0:8, :] = _pack(x_ref[pl.ds(base + 48, 16), :])
            h32_ref[12:16, :] = _pack(x_ref[pl.ds(base + 40, 8), :])
            Bs['hh'] = _unpack(h32_ref[...])
        NP = GW // PW
        n_mid_slots = 3 * NG * NP
        n_mid = NTILES - A_HEAD - 3 * A_TAIL
        slot = [0, 0]

        def proj_all(g, which):
            for piece in range(NP):
                proj1(g, which, piece)
                slot[0] += 1
                tgt = (n_mid * slot[0]) // n_mid_slots
                a_tiles(tgt - slot[1])
                slot[1] = tgt

        a_tiles(A_HEAD)
        proj_all(0, 'q'); proj_all(0, 'k'); proj_all(0, 'v')
        prep_next()
        for g in range(NG):
            last = g + 1 == NG
            b_scores(g)
            if not last:
                proj_all(g + 1, 'q')
            else:
                a_tiles(A_TAIL)
            b_softmax()
            b_pv(g)
            if not last:
                proj_all(g + 1, 'k')
            else:
                a_tiles(A_TAIL)
            b_norm(g)
            b_wo(g)
            if not last:
                proj_all(g + 1, 'v')
            else:
                a_tiles(A_TAIL)
        outb = Bs['acc'].astype(bf16)
        if parity == 0:
            b_ref[pl.ds(base + 16, 16), :] = outb[0:16, :]
            h32_ref[8:12, :] = _pack(outb[16:24, :])
            b_ref[pl.ds(base + 8, 8), :] = outb[24:32, :]
        else:
            b_ref[pl.ds(base + 48, 16), :] = outb[0:16, :]
            h48_ref[16:20, :] = _pack(outb[16:24, :])
            b_ref[pl.ds(base + 40, 8), :] = outb[24:32, :]
            b_ref[pl.ds(base, 8), :] = outb[32:40, :]
            b_ref[pl.ds(base + 32, 8), :] = outb[40:48, :]
        a_final()

    def body(t, carry):
        base = pl.multiple_of(t * (2 * SEG), 2 * SEG)
        t_next = jnp.minimum(t + 1, HA - 1)
        half_step(0, base, make_a_unit(t, 0), lambda: build_qm(t, 1))
        half_step(1, base, make_a_unit(t, 1), lambda: build_qm(t_next, 0))
        return carry

    build_qm(0, 0)
    jax.lax.fori_loop(0, S // (2 * SEG), body, 0)

    cp_awo.wait()
    awo = awo_ref[...]
    gw = gw_ref[...].astype(f32)
    outs = []
    for r in range(S // 128):
        rows = slice(r * 128, (r + 1) * 128)
        oa = oT_ref[:, rows].T.astype(bf16)
        a = jnp.dot(oa, awo, preferred_element_type=f32).astype(bf16).astype(f32)
        logit = jnp.sum(x_ref[rows, :].astype(f32) * gw, axis=-1, keepdims=True)
        gate = 1.0 / (1.0 + jnp.exp(-logit))
        ob_ref[rows, :] = (gate * a + (1.0 - gate) * b_ref[rows, :].astype(f32)).astype(bf16)
        cp = pltpu.make_async_copy(ob_ref.at[rows, :], out_hbm.at[rows, :], osems.at[r])
        cp.start()
        outs.append(cp)
    for cp in outs:
        cp.wait()


TQ, TW, KB, HG, LA = 1024, 128, 128, 8, 12
PVD = 0
PW, A_HEAD, A_TAIL = 128, 8, 8


@functools.partial(jax.jit, static_argnames=("B_seg_len",))
def pallas_gated_mix__mha_block__memory_aug_recurrent_mem_tr__prompt_kernel(
    A_x: jax.Array,
    A_wqkv: jax.Array,
    A_wo: jax.Array,
    B_x: jax.Array,
    B_mem0: jax.Array,
    B_Wq: jax.Array,
    B_Wk: jax.Array,
    B_Wv: jax.Array,
    B_Wo: jax.Array,
    B_seg_len: int,
    gate_w: jax.Array,
):
    Bsz, S, D = A_x.shape
    HA, DHA = 32, D // 32
    HB, DHB = B_Wq.shape[1], B_Wq.shape[2]
    M = B_mem0.shape[1]
    SEG = int(B_seg_len)
    assert Bsz == 1 and DHA == 16 and DHB == 128 and M == 8 and SEG == 32
    assert S == 2 * TQ and HA * (S // TQ) == S // SEG and HB % HG == 0
    R = 48

    x = A_x.reshape(S, D)
    mem0 = B_mem0.reshape(M, D)
    wq = B_Wq.reshape(D * HB, DHB)
    wk = B_Wk.reshape(D * HB, DHB)
    wv = B_Wv.reshape(D * HB, DHB)
    wo = B_Wo.reshape(HB * DHB, D)
    gw = gate_w.reshape(1, D)

    kernel = functools.partial(_kernel, S=S, D=D, HA=HA, DHA=DHA, HB=HB, DHB=DHB, SEG=SEG,
                               TQ=TQ, TW=TW, KB=KB, HG=HG, LA=LA, PW=PW, A_HEAD=A_HEAD, A_TAIL=A_TAIL, PVD=PVD)
    hbm = pl.BlockSpec(memory_space=pl.ANY)
    vmem = pl.BlockSpec(memory_space=pltpu.VMEM)
    out = pl.pallas_call(
        kernel,
        out_shape=jax.ShapeDtypeStruct((S, D), bf16),
        in_specs=[hbm, hbm, hbm, vmem, hbm, hbm, hbm, hbm, vmem],
        out_specs=hbm,
        scratch_shapes=[
            pltpu.VMEM((S, D), bf16),
            pltpu.VMEM((D, 3 * D), bf16),
            pltpu.VMEM((D, D), bf16),
            pltpu.VMEM((D * HB, DHB), bf16),
            pltpu.VMEM((D * HB, DHB), bf16),
            pltpu.VMEM((D * HB, DHB), bf16),
            pltpu.VMEM((HB * DHB, D), bf16),
            pltpu.SemaphoreType.DMA((7,)),
            pltpu.VMEM((S, D), bf16),
            pltpu.SemaphoreType.DMA((S // 128,)),
            pltpu.VMEM((S // 2, D), u32),
            pltpu.VMEM((D, S), bf16),
            pltpu.VMEM((D // 2, S), u32),
            pltpu.VMEM((D, S), f32),
            pltpu.VMEM((64, TQ), u32),
            pltpu.VMEM((64, TQ), u32),
            pltpu.VMEM((S, D), bf16),
            pltpu.VMEM((24, D), u32),
            pltpu.VMEM((16, D), u32),
            pltpu.VMEM((R // 2, HB * DHB), u32),
            pltpu.VMEM((R // 2, HB * DHB), u32),
            pltpu.VMEM((R // 2, HB * DHB), u32),
            pltpu.VMEM((R // 2, HB * DHB), u32),
            pltpu.VMEM((R // 2, HB * DHB), u32),
            pltpu.VMEM((D // 2, HB * DHB), u32),
            pltpu.VMEM((D // 2, HB * DHB), u32),
            pltpu.VMEM((D // 2, HB * DHB), u32),
            pltpu.VMEM((HB * DHB // 2, D), u32),
        ],
        compiler_params=pltpu.CompilerParams(vmem_limit_bytes=100 * 1024 * 1024),
    )(x, A_wqkv, A_wo, mem0, wq, wk, wv, wo, gw)
    return out.reshape(Bsz, S, D)
```
